```python
import jax
import jax.numpy as jnp

def _softmax(x, axis=-1):
    return jax.nn.softmax(x, axis=axis)
def _gelu(x):
    return jax.nn.gelu(x, approximate=True)
def _silu(x):
    return jax.nn.silu(x)
def _sigmoid(x):
    return jax.nn.sigmoid(x)
def _layernorm(x, axis=-1, eps=1e-5):
    m = jnp.mean(x, axis=axis, keepdims=True)
    v = jnp.var(x, axis=axis, keepdims=True)
    return (x - m) / jnp.sqrt(v + eps)
def _scatter_add(tgt, idx, src, axis=0):
    return tgt.at[idx].add(src)
def _segment_sum(src, seg, n):
    return jax.ops.segment_sum(src, seg, n)
class _Rng:
    def __init__(self, key):
        self._k = key
    def _next(self):
        self._k, sub = jax.random.split(self._k)
        return sub
    def normal(self, shape):
        return jax.random.normal(self._next(), shape, dtype=jnp.bfloat16)
    def randint(self, lo, hi, shape):
        return jax.random.randint(self._next(), shape, lo, hi, dtype=jnp.int32)
    def uniform(self, shape, lo=0.0, hi=1.0):
        return jax.random.uniform(self._next(), shape, jnp.bfloat16, lo, hi)
    def permutation(self, n):
        return jax.random.permutation(self._next(), n)


kernel_name = 'gated_mix__mha_block_cached__compressed_kv_cla__decode'

def setup_inputs():
    _rng = _Rng(jax.random.key(int.from_bytes(__import__("os").urandom(4), "little")))
    _w = (lambda a: (lambda t: t.astype(jnp.bfloat16) if jnp.issubdtype(t.dtype, jnp.floating) else t)(jnp.asarray(a)))
    def _A_setup():
        B, Sq, D = 2, 1, 512
        H, Sk, Dh = 32, 8192, 128
        return {
            "x": _w((lambda *s: _rng.normal(s) * 0.05)(B, Sq, D)),
            "k_cache": _w((lambda *s: _rng.normal(s) * 0.05)(B, H, Sk, Dh)),
            "v_cache": _w((lambda *s: _rng.normal(s) * 0.05)(B, H, Sk, Dh)),
            "wq": _w((lambda *s: _rng.normal(s) * 0.05)(D, H * Dh) * (D ** -0.5)),
            "wo": _w((lambda *s: _rng.normal(s) * 0.05)(H * Dh, D) * ((H * Dh) ** -0.5)),
        }
    _A_in = _A_setup()

    def _B_setup():
        B, H, Sq, Sk, D, M = 2, 32, 1, 8192, 128, 512
        Dc = 4 * D
        return {
            "x": _w((lambda *s: _rng.normal(s) * 0.05)(B, Sq, M)),
            "c_kv": _w((lambda *s: _rng.normal(s) * 0.05)(B, Sk, Dc)),
            "w_q": _w((lambda *s: _rng.normal(s) * 0.05)(M, H, D) * (M ** -0.5)),
            "w_uk": _w((lambda *s: _rng.normal(s) * 0.05)(Dc, H, D) * (Dc ** -0.5)),
            "w_uv": _w((lambda *s: _rng.normal(s) * 0.05)(Dc, H, D) * (Dc ** -0.5)),
            "w_o": _w((lambda *s: _rng.normal(s) * 0.05)(H, D, M) * ((H * D) ** -0.5)),
        }
    _B_in = _B_setup()

    return {
        "A_x": _A_in["x"],
        "A_k_cache": _A_in["k_cache"],
        "A_v_cache": _A_in["v_cache"],
        "A_wq": _A_in["wq"],
        "A_wo": _A_in["wo"],
        "B_x": _B_in["x"],
        "B_c_kv": _B_in["c_kv"],
        "B_w_q": _B_in["w_q"],
        "B_w_uk": _B_in["w_uk"],
        "B_w_uv": _B_in["w_uv"],
        "B_w_o": _B_in["w_o"],
        "gate_w": _w((lambda *s: _rng.normal(s) * 0.05)(512)),
    }

def reference(A_x, A_k_cache, A_v_cache, A_wq, A_wo, B_x, B_c_kv, B_w_q, B_w_uk, B_w_uv, B_w_o, gate_w):
    def _A_ref(x, k_cache, v_cache, wq, wo):
        B, Sq, D = x.shape
        H, Dh = 32, 128
        q = (lambda x, *d: x.transpose(*d))((x @ wq).reshape(B, Sq, H, Dh), 0, 2, 1, 3)
        scores = jnp.einsum("bhqd,bhkd->bhqk", q, k_cache) * (Dh ** -0.5)
        p = _softmax(scores, axis=-1)
        o = jnp.einsum("bhqk,bhkd->bhqd", p, v_cache)
        return (lambda x, *d: x.transpose(*d))(o, 0, 2, 1, 3).reshape(B, Sq, H * Dh) @ wo

    def _B_ref(x, c_kv, w_q, w_uk, w_uv, w_o):
        B, Sq, M = x.shape[0], x.shape[1], x.shape[2]
        Sk = c_kv.shape[1]
        H, D = w_q.shape[1], w_q.shape[2]
        q = jnp.einsum("bqm,mhd->bhqd", x, w_q)
        k = jnp.einsum("bkc,chd->bhkd", c_kv, w_uk)
        v = jnp.einsum("bkc,chd->bhkd", c_kv, w_uv)
        scores = jnp.einsum("bhqd,bhkd->bhqk", q, k) * (D ** -0.5)
        off = Sk - Sq
        qi = jnp.arange(Sq)[:, None]
        kj = jnp.arange(Sk)[None, :]
        cmask = kj <= (qi + off)
        scores = jnp.where(cmask[None, None], scores, -1e9)
        p = _softmax(scores, axis=-1)
        ctx = jnp.einsum("bhqk,bhkd->bhqd", p, v)
        return jnp.einsum("bhqd,hdm->bqm", ctx, w_o)

    x = A_x
    g = _sigmoid((x * gate_w).sum(-1, keepdims=True))
    a = _A_ref(x, A_k_cache, A_v_cache, A_wq, A_wo)
    b = _B_ref(x, B_c_kv, B_w_q, B_w_uk, B_w_uv, B_w_o)
    return g * a + (1 - g) * b
```

```python
import functools

import jax
import jax.numpy as jnp
import jax.experimental.pallas as pl
import jax.experimental.pallas.tpu as pltpu

_B, _H, _SK, _DH, _D, _DC = 2, 32, 8192, 128, 512, 512

_PIECE_ROWS = 128
_PRIO = (0, 1, 1, 1)
_NSLOT = 2

_f32 = jnp.float32
_bf16 = jnp.bfloat16


def _dot(a, b):
    return jnp.dot(a, b, preferred_element_type=_f32)


def _dot_t(a, b):
    return jax.lax.dot_general(a, b, (((1,), (1,)), ((), ())), preferred_element_type=_f32)


def _unpack_pair(blk):
    lo = pltpu.bitcast(blk << 16, _f32).astype(_bf16)
    hi = pltpu.bitcast(blk & jnp.int32(-65536), _f32).astype(_bf16)
    return lo, hi


def _kernel(x_ref, gw_ref,
            k_hbm, v_hbm, wq_hbm, wo_hbm, ckv_hbm, bwq_hbm, bwuk_hbm, bwuv_hbm, bwo_hbm,
            out_ref,
            kv_buf, wq_v, wo_v, ckv_v, bwq_v, bwuk_v, bwuv_v, bwo_v,
            qa_s, qb_s, qlat_s, clat_s, o_s, ctx_s, m_s, l_s, acc_s,
            kv_sem, w_sem):

    def row_pieces(src, dst, rows, r0, n, sem, src_off=0):
        for p in range(r0, r0 + n):
            pltpu.make_async_copy(
                src.at[pl.ds(src_off + p * rows, rows)], dst.at[pl.ds(p * rows, rows)], sem
            ).start(priority=_PRIO[p % len(_PRIO)])

    def wait_all(dst, sem):
        pltpu.make_async_copy(dst, dst, sem).wait()

    def start_wq(lo, hi):
        for p in range(lo, hi):
            r, c = p // 4, p % 4
            pltpu.make_async_copy(
                wq_hbm.at[pl.ds(r * 16, 16), pl.ds(c * 1024, 1024)],
                wq_v.at[pl.ds(r * 16, 16), pl.ds(c * 1024, 1024)], w_sem.at[0]
            ).start(priority=_PRIO[p % len(_PRIO)])

    def start_kv(i, slot):
        bh = (i % 2) * _H + i // 2
        for p in range(2 * _SK // _PIECE_ROWS):
            src = (k_hbm, v_hbm)[p % 2]
            r = (p // 2) * _PIECE_ROWS
            pltpu.make_async_copy(
                src.at[bh, pl.ds(r, _PIECE_ROWS)],
                kv_buf.at[slot, p % 2, pl.ds(r, _PIECE_ROWS)], kv_sem.at[slot]
            ).start(priority=_PRIO[p % len(_PRIO)])

    S_WQ, S_BWQ, S_BWUK, S_BWUV, S_WO, S_BWO = 0, 1, 2, 3, 4, 5
    S_CKV = 6
    S_BWO2 = 14
    NCK = 8
    CK = _B * _SK // NCK

    def start_ckv(c):
        row_pieces(ckv_hbm, ckv_v.at[c], 32, 0, CK // 32, w_sem.at[S_CKV + c], src_off=c * CK)

    row8 = jax.lax.broadcasted_iota(jnp.int32, (8, _D), 0)
    scale_a = _DH ** -0.5
    scale_b = _DH ** -0.5

    def load_x8():
        xf = x_ref[...].astype(_f32)
        x0 = xf[0]
        x1 = xf[1]
        return jnp.where(row8 == 0, x0, jnp.where(row8 == 1, x1, 0.0))

    def compute_qa(x8):
        q = _dot(x8, wq_v[...]) * scale_a
        for h in range(_H):
            qa_s[h] = q[:, h * _DH:(h + 1) * _DH]

    def compute_qb(x8, i0, i1):
        w32 = bwq_v.bitcast(jnp.int32)
        for i in range(i0, i1):
            lo, hi = _unpack_pair(w32[pl.ds(i, _D, stride=_H // 2), :])
            qb_s[2 * i] = _dot(x8, lo)
            qb_s[2 * i + 1] = _dot(x8, hi)

    def compute_qlat(i0, i1):
        w32 = bwuk_v.bitcast(jnp.int32)
        for i in range(i0, i1):
            pair = _unpack_pair(w32[pl.ds(i, _DC, stride=_H // 2), :])
            for j in range(2):
                h = 2 * i + j
                ql = _dot_t(qb_s[h].astype(_bf16), pair[j]) * scale_b
                qlat_s[0, pl.ds(h, 1), :] = ql[0:1, :]
                qlat_s[1, pl.ds(h, 1), :] = ql[1:2, :]

    def b_chunk(c):
        b = c // (NCK // _B)
        first = c % (NCK // _B) == 0
        last = c % (NCK // _B) == NCK // _B - 1
        ck = ckv_v[c]
        s = _dot_t(qlat_s[b].astype(_bf16), ck)
        m_cur = jnp.max(s, axis=-1, keepdims=True)
        if first:
            m_new = m_cur
        else:
            m_old = m_s[...]
            m_new = jnp.maximum(m_old, m_cur)
        p = jnp.exp(s - m_new)
        l_cur = jnp.sum(p, axis=-1, keepdims=True)
        pv = _dot(p.astype(_bf16), ck)
        if first:
            l_new, acc = l_cur, pv
        else:
            alpha = jnp.exp(m_old - m_new)
            l_new = alpha * l_s[...] + l_cur
            acc = alpha * acc_s[...] + pv
        if last:
            clat_s[b] = acc / l_new
        else:
            m_s[...] = m_new
            l_s[...] = l_new
            acc_s[...] = acc

    def compute_ctx(i0, i1):
        w32 = bwuv_v.bitcast(jnp.int32)
        for i in range(i0, i1):
            pair = _unpack_pair(w32[pl.ds(i, _DC, stride=_H // 2), :])
            for j in range(2):
                h = 2 * i + j
                r0 = clat_s[0, pl.ds(h, 1), :]
                r1 = clat_s[1, pl.ds(h, 1), :]
                lhs = jnp.where(row8 == 0, r0, jnp.where(row8 == 1, r1, 0.0))
                ctx_s[h] = _dot(lhs.astype(_bf16), pair[j])

    row8h = jax.lax.broadcasted_iota(jnp.int32, (8, _DH), 0)

    def a_head(i, slot):
        b = i % 2
        h = i // 2
        q8 = qa_s[h].astype(_bf16)
        s = _dot_t(q8, kv_buf[slot, 0])
        m = jnp.max(s, axis=-1, keepdims=True)
        p = jnp.exp(s - m)
        l = jnp.sum(p, axis=-1, keepdims=True)
        o = _dot(p.astype(_bf16), kv_buf[slot, 1]) / l
        o_s[h] = jnp.where(row8h == b, o, o_s[h])

    def out_proj(src_s, w_v, h0, h1):
        acc = None
        for h in range(h0, h1):
            t = _dot(src_s[h].astype(_bf16), w_v[pl.ds(h * _DH, _DH), :])
            acc = t if acc is None else acc + t
        return acc

    start_wq(0, 128)
    o_s[...] = jnp.zeros_like(o_s)
    x8f = load_x8()
    x8 = x8f.astype(_bf16)

    row_pieces(bwq_hbm, bwq_v, 128, 0, 128, w_sem.at[S_BWQ])
    wait_all(wq_v, w_sem.at[S_WQ])
    compute_qa(x8)

    row_pieces(bwuk_hbm, bwuk_v, 128, 0, 64, w_sem.at[S_BWUK])
    wait_all(bwq_v, w_sem.at[S_BWQ])
    compute_qb(x8, 0, 8)
    row_pieces(bwuk_hbm, bwuk_v, 128, 64, 64, w_sem.at[S_BWUK])
    compute_qb(x8, 8, 16)

    start_ckv(0)
    wait_all(bwuk_v, w_sem.at[S_BWUK])
    compute_qlat(0, 8)
    start_ckv(1)
    compute_qlat(8, 16)

    for c in range(NCK):
        if c + 2 < NCK:
            start_ckv(c + 2)
        elif c + 2 == NCK:
            row_pieces(bwuv_hbm, bwuv_v, 128, 0, 64, w_sem.at[S_BWUV])
        else:
            row_pieces(bwuv_hbm, bwuv_v, 128, 64, 64, w_sem.at[S_BWUV])
        wait_all(ckv_v.at[c], w_sem.at[S_CKV + c])
        b_chunk(c)

    start_kv(0, 0)
    wait_all(bwuv_v, w_sem.at[S_BWUV])
    compute_ctx(0, 16)

    nbh = _B * _H

    def body(it, carry):
        for s in range(_NSLOT):
            i = it * _NSLOT + s
            nxt = (s + 1) % _NSLOT
            start_kv(i + 1, nxt)
            wait_all(kv_buf.at[s], kv_sem.at[s])
            a_head(i, s)
        return carry

    n_main = (nbh - 1) // _NSLOT
    jax.lax.fori_loop(0, n_main, body, 0)
    for i in range(n_main * _NSLOT, nbh):
        s = i % _NSLOT
        if i + 1 < nbh:
            start_kv(i + 1, (i + 1) % _NSLOT)
        else:
            row_pieces(wo_hbm, wo_v, 32, 0, 128, w_sem.at[S_WO])
        wait_all(kv_buf.at[s], kv_sem.at[s])
        a_head(i, s)

    row_pieces(bwo_hbm, bwo_v, 32, 0, 64, w_sem.at[S_BWO])
    wait_all(wo_v, w_sem.at[S_WO])
    row_pieces(bwo_hbm, bwo_v, 32, 64, 64, w_sem.at[S_BWO2])
    out_a = out_proj(o_s, wo_v, 0, _H)
    gate = jax.nn.sigmoid(jnp.sum(x8f * gw_ref[...].astype(_f32), axis=-1, keepdims=True))
    wait_all(bwo_v.at[pl.ds(0, 2048)], w_sem.at[S_BWO])
    out_b = out_proj(ctx_s, bwo_v, 0, _H // 2)
    wait_all(bwo_v.at[pl.ds(2048, 2048)], w_sem.at[S_BWO2])
    out_b = out_b + out_proj(ctx_s, bwo_v, _H // 2, _H)
    res = (gate * out_a + (1.0 - gate) * out_b).astype(_bf16)
    out_ref[0] = res[0:1, :]
    out_ref[1] = res[1:2, :]


@jax.jit
def pallas_gated_mix__mha_block_cached__compressed_kv_cla__decode_kernel(
    A_x: jax.Array,
    A_k_cache: jax.Array,
    A_v_cache: jax.Array,
    A_wq: jax.Array,
    A_wo: jax.Array,
    B_x: jax.Array,
    B_c_kv: jax.Array,
    B_w_q: jax.Array,
    B_w_uk: jax.Array,
    B_w_uv: jax.Array,
    B_w_o: jax.Array,
    gate_w: jax.Array,
):
    del B_x
    k3 = A_k_cache.reshape(_B * _H, _SK, _DH)
    v3 = A_v_cache.reshape(_B * _H, _SK, _DH)
    ckv = B_c_kv.reshape(_B * _SK, _DC)
    bwq = B_w_q.reshape(_D * _H, _DH)
    bwuk = B_w_uk.reshape(_DC * _H, _DH)
    bwuv = B_w_uv.reshape(_DC * _H, _DH)
    bwo = B_w_o.reshape(_H * _DH, _D)
    gw = gate_w.reshape(1, _D)

    hbm = pl.BlockSpec(memory_space=pl.ANY)
    vmem = pl.BlockSpec(memory_space=pltpu.VMEM)
    V = pltpu.VMEM
    scratch = [
        V((_NSLOT, 2, _SK, _DH), _bf16),
        V((_D, _H * _DH), _bf16),
        V((_H * _DH, _D), _bf16),
        V((8, _B * _SK // 8, _DC), _bf16),
        V((_D * _H, _DH), _bf16),
        V((_DC * _H, _DH), _bf16),
        V((_DC * _H, _DH), _bf16),
        V((_H * _DH, _D), _bf16),
        V((_H, 8, _DH), _f32),
        V((_H, 8, _DH), _f32),
        V((_B, _H, _DC), _f32),
        V((_B, _H, _DC), _f32),
        V((_H, 8, _DH), _f32),
        V((_H, 8, _DH), _f32),
        V((_H, 1), _f32),
        V((_H, 1), _f32),
        V((_H, _DC), _f32),
        pltpu.SemaphoreType.DMA((_NSLOT,)),
        pltpu.SemaphoreType.DMA((15,)),
    ]
    return pl.pallas_call(
        _kernel,
        out_shape=jax.ShapeDtypeStruct((_B, 1, _D), _bf16),
        in_specs=[vmem, vmem] + [hbm] * 9,
        out_specs=vmem,
        scratch_shapes=scratch,
        compiler_params=pltpu.CompilerParams(vmem_limit_bytes=100 * 1024 * 1024),
    )(A_x, gw, k3, v3, A_wq, A_wo, ckv, bwq, bwuk, bwuv, bwo)
```

```python
import functools

import jax
import jax.numpy as jnp
import jax.experimental.pallas as pl
import jax.experimental.pallas.tpu as pltpu

_B, _H, _SK, _DH, _D, _DC = 2, 32, 8192, 128, 512, 512

_PIECE_ROWS = 128
_PRIO = (0, 1, 1, 1)
_NCK = 8
_END = (8, 8, 8, 4, 2, 2)
_AHEAD = (1, 1, 9, 9, 9, 9)
_NPEEL = 4
_NSLOT = 2

_f32 = jnp.float32
_bf16 = jnp.bfloat16


def _dot(a, b):
    return jnp.dot(a, b, preferred_element_type=_f32)


def _dot_t(a, b):
    return jax.lax.dot_general(a, b, (((1,), (1,)), ((), ())), preferred_element_type=_f32)


def _unpack_pair(blk):
    lo = pltpu.bitcast(blk << 16, _f32).astype(_bf16)
    hi = pltpu.bitcast(blk & jnp.int32(-65536), _f32).astype(_bf16)
    return lo, hi


def _kernel(x_hbm, gw_hbm,
            k_hbm, v_hbm, wq_hbm, wo_hbm, ckv_hbm, bwq_hbm, bwuk_hbm, bwuv_hbm, bwo_hbm,
            out_ref,
            kv_buf, wq_v, wo_v, ckv_v, bwq_v, bwuk_v, bwuv_v, bwo_v,
            qa_s, qb_s, qlat_s, clat_s, o_s, ctx_s, m_s, l_s, acc_s,
            x_ref, gw_ref, kv_sem, w_sem, x_sem):

    def rows(src, dst, nrow, n, sem, soff=0, doff=0):
        return [(src.at[pl.ds(soff + p * nrow, nrow)], dst.at[pl.ds(doff + p * nrow, nrow)], sem)
                for p in range(n)]

    def zip2(u, v):
        out = []
        for a, b in zip(u, v):
            out += [a, b]
        return out

    def issue(unit, lo=0, hi=None):
        for p in range(lo, len(unit) if hi is None else hi):
            src, dst, sem = unit[p]
            pltpu.make_async_copy(src, dst, sem).start(priority=_PRIO[p % len(_PRIO)])

    def wait_all(dst, sem):
        pltpu.make_async_copy(dst, dst, sem).wait()

    S_WQ, S_BWQ, S_BWUK, S_BWUV = 0, 1, 2, 3
    S_CKV = 4
    NCK = _NCK
    CK = _SK // NCK
    S_END = S_CKV + 2 * NCK

    u_wq = [(wq_hbm.at[pl.ds((p // 4) * 16, 16), pl.ds((p % 4) * 1024, 1024)],
             wq_v.at[pl.ds((p // 4) * 16, 16), pl.ds((p % 4) * 1024, 1024)], w_sem.at[S_WQ])
            for p in range(128)]
    u_w1 = zip2(u_wq, rows(bwq_hbm, bwq_v, 128, 128, w_sem.at[S_BWQ]))
    u_w2 = zip2(rows(bwuk_hbm, bwuk_v, 128, 128, w_sem.at[S_BWUK]),
                rows(bwuv_hbm, bwuv_v, 128, 128, w_sem.at[S_BWUV]))

    def u_ckv(c):
        return zip2(*[rows(ckv_hbm, ckv_v.at[b * NCK + c], 32, CK // 32, w_sem.at[S_CKV + b * NCK + c],
                           soff=b * _SK + c * CK) for b in range(_B)])

    end_h = [0]
    for n in _END:
        end_h.append(end_h[-1] + n)

    def u_end(e):
        h0, n = end_h[e], _END[e]
        return zip2(*[rows(src, dst, 32, n * _DH // 32, w_sem.at[S_END + e], soff=h0 * _DH, doff=h0 * _DH)
                      for src, dst in ((wo_hbm, wo_v), (bwo_hbm, bwo_v))])

    def u_kv(i, slot):
        bh = (i % 2) * _H + i // 2
        n = _SK // _PIECE_ROWS
        return [((k_hbm, v_hbm)[p % 2].at[bh, pl.ds((p // 2) * _PIECE_ROWS, _PIECE_ROWS)],
                 kv_buf.at[slot, p % 2, pl.ds((p // 2) * _PIECE_ROWS, _PIECE_ROWS)], kv_sem.at[slot])
                for p in range(2 * n)]

    row8 = jax.lax.broadcasted_iota(jnp.int32, (8, _D), 0)
    scale_a = _DH ** -0.5
    scale_b = _DH ** -0.5

    def load_x8():
        xf = x_ref[...].astype(_f32)
        x0 = xf[0:1]
        x1 = xf[1:2]
        return jnp.where(row8 == 0, x0, jnp.where(row8 == 1, x1, 0.0))

    def compute_qa(x8):
        q = _dot(x8, wq_v[...]) * scale_a
        for h in range(_H):
            qa_s[h] = q[:, h * _DH:(h + 1) * _DH]

    def compute_qb(x8, i0, i1):
        w32 = bwq_v.bitcast(jnp.int32)
        for i in range(i0, i1):
            lo, hi = _unpack_pair(w32[pl.ds(i, _D, stride=_H // 2), :])
            qb_s[2 * i] = _dot(x8, lo)
            qb_s[2 * i + 1] = _dot(x8, hi)

    def compute_qlat(i0, i1):
        w32 = bwuk_v.bitcast(jnp.int32)
        for i in range(i0, i1):
            pair = _unpack_pair(w32[pl.ds(i, _DC, stride=_H // 2), :])
            for j in range(2):
                h = 2 * i + j
                ql = _dot_t(qb_s[h].astype(_bf16), pair[j]) * scale_b
                qlat_s[0, pl.ds(h, 1), :] = ql[0:1, :]
                qlat_s[1, pl.ds(h, 1), :] = ql[1:2, :]

    def b_chunk(b, c):
        first = c == 0
        last = c == NCK - 1
        ck = ckv_v[b * NCK + c]
        s = _dot_t(qlat_s[b].astype(_bf16), ck)
        m_cur = jnp.max(s, axis=-1, keepdims=True)
        if first:
            m_new = m_cur
        else:
            m_old = m_s[b]
            m_new = jnp.maximum(m_old, m_cur)
        p = jnp.exp(s - m_new)
        l_cur = jnp.sum(p, axis=-1, keepdims=True)
        pv = _dot(p.astype(_bf16), ck)
        if first:
            l_new, acc = l_cur, pv
        else:
            alpha = jnp.exp(m_old - m_new)
            l_new = alpha * l_s[b] + l_cur
            acc = alpha * acc_s[b] + pv
        if last:
            clat_s[b] = acc / l_new
        else:
            m_s[b] = m_new
            l_s[b] = l_new
            acc_s[b] = acc

    def compute_ctx(i0, i1):
        w32 = bwuv_v.bitcast(jnp.int32)
        for i in range(i0, i1):
            pair = _unpack_pair(w32[pl.ds(i, _DC, stride=_H // 2), :])
            for j in range(2):
                h = 2 * i + j
                r0 = clat_s[0, pl.ds(h, 1), :]
                r1 = clat_s[1, pl.ds(h, 1), :]
                lhs = jnp.where(row8 == 0, r0, jnp.where(row8 == 1, r1, 0.0))
                ctx_s[h] = _dot(lhs.astype(_bf16), pair[j])

    row8h = jax.lax.broadcasted_iota(jnp.int32, (8, _DH), 0)

    def a_head(i, slot):
        b = i % 2
        h = i // 2
        q8 = qa_s[h].astype(_bf16)
        s = _dot_t(q8, kv_buf[slot, 0])
        m = jnp.max(s, axis=-1, keepdims=True)
        p = jnp.exp(s - m)
        l = jnp.sum(p, axis=-1, keepdims=True)
        o = _dot(p.astype(_bf16), kv_buf[slot, 1]) / l
        o_s[h] = jnp.where(row8h == b, o, o_s[h])

    def out_proj(src_s, w_v, h0, h1):
        acc = None
        for h in range(h0, h1):
            t = _dot(src_s[h].astype(_bf16), w_v[pl.ds(h * _DH, _DH), :])
            acc = t if acc is None else acc + t
        return acc

    cx = pltpu.make_async_copy(x_hbm, x_ref, x_sem.at[0])
    cg = pltpu.make_async_copy(gw_hbm, gw_ref, x_sem.at[1])
    cx.start()
    cg.start()
    issue(u_w1)
    o_s[...] = jnp.zeros_like(o_s)
    cx.wait()
    cg.wait()
    x8f = load_x8()
    x8 = x8f.astype(_bf16)
    gate = jax.nn.sigmoid(jnp.sum(x8f * gw_ref[...].astype(_f32).reshape(1, _D), axis=-1, keepdims=True))

    issue(u_w2, 0, 64)
    wait_all(wq_v, w_sem.at[S_WQ])
    compute_qa(x8)
    issue(u_w2, 64, 128)
    wait_all(bwq_v, w_sem.at[S_BWQ])
    compute_qb(x8, 0, 8)
    issue(u_w2, 128, 192)
    compute_qb(x8, 8, 16)
    issue(u_w2, 192, 256)

    ck = [u_ckv(c) for c in range(NCK)]
    half = len(ck[0]) // 2
    issue(ck[0])
    wait_all(bwuk_v, w_sem.at[S_BWUK])
    compute_qlat(0, 8)
    issue(ck[1])
    compute_qlat(8, 16)

    kv0 = u_kv(0, 0)
    nkv = len(kv0)
    for c in range(NCK):
        for b in range(_B):
            if c + 2 < NCK:
                issue(ck[c + 2], b * half, (b + 1) * half)
            else:
                t = (c + 2 - NCK) * _B + b
                issue(kv0, t * nkv // 4, (t + 1) * nkv // 4)
            wait_all(ckv_v.at[b * NCK + c], w_sem.at[S_CKV + b * NCK + c])
            b_chunk(b, c)

    nbh = _B * _H

    def step(i, s, extra=None):
        issue(u_kv(i + 1, (s + 1) % _NSLOT))
        wait_all(kv_buf.at[s], kv_sem.at[s])
        a_head(i, s)
        if extra is not None:
            extra()

    NPEEL = _NPEEL
    wait_all(bwuv_v, w_sem.at[S_BWUV])
    for i in range(NPEEL):
        step(i, i % _NSLOT, functools.partial(compute_ctx, i * 16 // NPEEL, (i + 1) * 16 // NPEEL))

    def body(it, carry):
        for s in range(_NSLOT):
            step(it * _NSLOT + s, s)
        return carry

    NE = len(_END)
    ue = [u_end(e) for e in range(NE)]
    n_main = (nbh - 1) // _NSLOT
    jax.lax.fori_loop(NPEEL // _NSLOT, n_main, body, 0)
    for i in range(n_main * _NSLOT, nbh):
        s = i % _NSLOT
        if i + 1 < nbh:
            issue(u_kv(i + 1, (i + 1) % _NSLOT))
        else:
            issue(ue[0])
        wait_all(kv_buf.at[s], kv_sem.at[s])
        a_head(i, s)

    out_a = None
    out_b = None
    nxt = 1
    for e in range(NE):
        while nxt < min(e + 1 + _AHEAD[e], NE):
            issue(ue[nxt])
            nxt += 1
        h0, h1 = end_h[e], end_h[e + 1]
        wait_all(wo_v.at[pl.ds(h0 * _DH, (h1 - h0) * _DH)], w_sem.at[S_END + e])
        wait_all(bwo_v.at[pl.ds(h0 * _DH, (h1 - h0) * _DH)], w_sem.at[S_END + e])
        ta = out_proj(o_s, wo_v, h0, h1)
        tb = out_proj(ctx_s, bwo_v, h0, h1)
        out_a = ta if out_a is None else out_a + ta
        out_b = tb if out_b is None else out_b + tb
    res = gate * out_a + (1.0 - gate) * out_b
    out_ref[...] = res[0:2, :].astype(_bf16)


@jax.jit
def pallas_gated_mix__mha_block_cached__compressed_kv_cla__decode_kernel(
    A_x: jax.Array,
    A_k_cache: jax.Array,
    A_v_cache: jax.Array,
    A_wq: jax.Array,
    A_wo: jax.Array,
    B_x: jax.Array,
    B_c_kv: jax.Array,
    B_w_q: jax.Array,
    B_w_uk: jax.Array,
    B_w_uv: jax.Array,
    B_w_o: jax.Array,
    gate_w: jax.Array,
):
    del B_x
    k3 = A_k_cache.reshape(_B * _H, _SK, _DH)
    v3 = A_v_cache.reshape(_B * _H, _SK, _DH)
    ckv = B_c_kv.reshape(_B * _SK, _DC)
    bwq = B_w_q.reshape(_D * _H, _DH)
    bwuk = B_w_uk.reshape(_DC * _H, _DH)
    bwuv = B_w_uv.reshape(_DC * _H, _DH)
    bwo = B_w_o.reshape(_H * _DH, _D)
    x2 = A_x.reshape(_B, _D)

    hbm = pl.BlockSpec(memory_space=pl.ANY)
    vmem = pl.BlockSpec(memory_space=pltpu.VMEM)
    V = pltpu.VMEM
    scratch = [
        V((_NSLOT, 2, _SK, _DH), _bf16),
        V((_D, _H * _DH), _bf16),
        V((_H * _DH, _D), _bf16),
        V((_B * _NCK, _SK // _NCK, _DC), _bf16),
        V((_D * _H, _DH), _bf16),
        V((_DC * _H, _DH), _bf16),
        V((_DC * _H, _DH), _bf16),
        V((_H * _DH, _D), _bf16),
        V((_H, 8, _DH), _f32),
        V((_H, 8, _DH), _f32),
        V((_B, _H, _DC), _f32),
        V((_B, _H, _DC), _f32),
        V((_H, 8, _DH), _f32),
        V((_H, 8, _DH), _f32),
        V((_B, _H, 1), _f32),
        V((_B, _H, 1), _f32),
        V((_B, _H, _DC), _f32),
        V((_B, _D), _bf16),
        V((_D,), _bf16),
        pltpu.SemaphoreType.DMA((_NSLOT,)),
        pltpu.SemaphoreType.DMA((4 + 2 * _NCK + len(_END),)),
        pltpu.SemaphoreType.DMA((2,)),
    ]
    out = pl.pallas_call(
        _kernel,
        out_shape=jax.ShapeDtypeStruct((_B, _D), _bf16),
        in_specs=[hbm] * 11,
        out_specs=vmem,
        scratch_shapes=scratch,
        compiler_params=pltpu.CompilerParams(vmem_limit_bytes=100 * 1024 * 1024),
    )(x2, gate_w, k3, v3, A_wq, A_wo, ckv, bwq, bwuk, bwuv, bwo)
    return out.reshape(_B, 1, _D)
```

```python
import functools

import jax
import jax.numpy as jnp
import jax.experimental.pallas as pl
import jax.experimental.pallas.tpu as pltpu

_B, _H, _SK, _DH, _D, _DC = 2, 32, 8192, 128, 512, 512

_PIECE_ROWS = 128
_PRIO_KV, _RUN_KV = (0, 1), 1
_ROT_KV = 2
_ROT_W = 2
_ROT_C = 2
_ROT_E = 2
_PRIO_W, _RUN_W = (0, 1), 1
_PRIO_C, _RUN_C = (0, 1), 1
_PRIO_E, _RUN_E = (0, 1), 1
_NCK = 8
_END = (8, 8, 8, 4, 2, 2)
_AHEAD = (1, 1, 9, 9, 9, 9)
_NPEEL = 4
_NSLOT = 2

_f32 = jnp.float32
_bf16 = jnp.bfloat16


def _dot(a, b):
    return jnp.dot(a, b, preferred_element_type=_f32)


def _dot_t(a, b):
    return jax.lax.dot_general(a, b, (((1,), (1,)), ((), ())), preferred_element_type=_f32)


def _unpack_pair(blk):
    lo = pltpu.bitcast(blk << 16, _f32).astype(_bf16)
    hi = pltpu.bitcast(blk & jnp.int32(-65536), _f32).astype(_bf16)
    return lo, hi


def _kernel(x_hbm, gw_hbm,
            k_hbm, v_hbm, wq_hbm, wo_hbm, ckv_hbm, bwq_hbm, bwuk_hbm, bwuv_hbm, bwo_hbm,
            out_ref,
            kv_buf, wq_v, wo_v, ckv_v, bwq_v, bwuk_v, bwuv_v, bwo_v,
            qa_s, qb_s, qlat_s, clat_s, o_s, ctx_s, m_s, l_s, acc_s,
            x_ref, gw_ref, kv_sem, w_sem, x_sem):

    def rows(src, dst, nrow, n, sem, soff=0, doff=0):
        return [(src.at[pl.ds(soff + p * nrow, nrow)], dst.at[pl.ds(doff + p * nrow, nrow)], sem)
                for p in range(n)]

    def rot(u, mode):
        n = len(u)
        if mode == 0:
            return u
        if n % 64 == 0:
            if mode == 2:
                return [u[(p // 64) * 64 + (p % 4) * 16 + (p % 64) // 4] for p in range(n)]
            return [u[(p // 64) * 64 + (p % 2) * 32 + (p % 64) // 2] for p in range(n)]
        if n % 32 == 0:
            return [u[(p // 32) * 32 + (p % 2) * 16 + (p % 32) // 2] for p in range(n)]
        return u

    def zip2(u, v, run=_RUN_W, prio=_PRIO_W, mode=_ROT_W):
        u, v = rot(u, mode), rot(v, mode)
        out = []
        for j in range(0, len(u), run):
            out += u[j:j + run] + v[j:j + run]
        return [(a, b, c, prio[p % len(prio)]) for p, (a, b, c) in enumerate(out)]

    def issue(unit, lo=0, hi=None):
        for p in range(lo, len(unit) if hi is None else hi):
            src, dst, sem, prio = unit[p]
            pltpu.make_async_copy(src, dst, sem).start(priority=prio)

    def wait_all(dst, sem):
        pltpu.make_async_copy(dst, dst, sem).wait()

    S_WQ, S_BWQ, S_BWUK, S_BWUV = 0, 1, 2, 3
    S_CKV = 4
    NCK = _NCK
    CK = _SK // NCK
    S_END = S_CKV + 2 * NCK

    u_wq = [(wq_hbm.at[pl.ds((p // 4) * 16, 16), pl.ds((p % 4) * 1024, 1024)],
             wq_v.at[pl.ds((p // 4) * 16, 16), pl.ds((p % 4) * 1024, 1024)], w_sem.at[S_WQ])
            for p in range(128)]
    u_w1 = zip2(u_wq, rows(bwq_hbm, bwq_v, 128, 128, w_sem.at[S_BWQ]))
    u_w2 = zip2(rows(bwuk_hbm, bwuk_v, 128, 128, w_sem.at[S_BWUK]),
                rows(bwuv_hbm, bwuv_v, 128, 128, w_sem.at[S_BWUV]))

    def u_ckv(c):
        return zip2(*[rows(ckv_hbm, ckv_v.at[b * NCK + c], 32, CK // 32, w_sem.at[S_CKV + b * NCK + c],
                           soff=b * _SK + c * CK) for b in range(_B)], run=_RUN_C, prio=_PRIO_C, mode=_ROT_C)

    end_h = [0]
    for n in _END:
        end_h.append(end_h[-1] + n)

    def u_end(e):
        h0, n = end_h[e], _END[e]
        return zip2(*[rows(src, dst, 32, n * _DH // 32, w_sem.at[S_END + e], soff=h0 * _DH, doff=h0 * _DH)
                      for src, dst in ((wo_hbm, wo_v), (bwo_hbm, bwo_v))], run=_RUN_E, prio=_PRIO_E, mode=_ROT_E)

    def u_kv(i, slot):
        bh = (i % 2) * _H + i // 2
        n = _SK // _PIECE_ROWS
        return zip2(*[[(src.at[bh, pl.ds(p * _PIECE_ROWS, _PIECE_ROWS)],
                        kv_buf.at[slot, j, pl.ds(p * _PIECE_ROWS, _PIECE_ROWS)], kv_sem.at[slot])
                       for p in range(n)] for j, src in enumerate((k_hbm, v_hbm))], run=_RUN_KV, prio=_PRIO_KV, mode=_ROT_KV)

    row8 = jax.lax.broadcasted_iota(jnp.int32, (8, _D), 0)
    scale_a = _DH ** -0.5
    scale_b = _DH ** -0.5

    def load_x8():
        xf = x_ref[...].astype(_f32)
        x0 = xf[0:1]
        x1 = xf[1:2]
        return jnp.where(row8 == 0, x0, jnp.where(row8 == 1, x1, 0.0))

    def compute_qa(x8):
        q = _dot(x8, wq_v[...]) * scale_a
        for h in range(_H):
            qa_s[h] = q[:, h * _DH:(h + 1) * _DH]

    def compute_qb(x8, i0, i1):
        w32 = bwq_v.bitcast(jnp.int32)
        for i in range(i0, i1):
            lo, hi = _unpack_pair(w32[pl.ds(i, _D, stride=_H // 2), :])
            qb_s[2 * i] = _dot(x8, lo)
            qb_s[2 * i + 1] = _dot(x8, hi)

    def compute_qlat(i0, i1):
        w32 = bwuk_v.bitcast(jnp.int32)
        for i in range(i0, i1):
            pair = _unpack_pair(w32[pl.ds(i, _DC, stride=_H // 2), :])
            for j in range(2):
                h = 2 * i + j
                ql = _dot_t(qb_s[h].astype(_bf16), pair[j]) * scale_b
                qlat_s[0, pl.ds(h, 1), :] = ql[0:1, :]
                qlat_s[1, pl.ds(h, 1), :] = ql[1:2, :]

    def b_chunk(b, c):
        first = c == 0
        last = c == NCK - 1
        ck = ckv_v[b * NCK + c]
        s = _dot_t(qlat_s[b].astype(_bf16), ck)
        m_cur = jnp.max(s, axis=-1, keepdims=True)
        if first:
            m_new = m_cur
        else:
            m_old = m_s[b]
            m_new = jnp.maximum(m_old, m_cur)
        p = jnp.exp(s - m_new)
        l_cur = jnp.sum(p, axis=-1, keepdims=True)
        pv = _dot(p.astype(_bf16), ck)
        if first:
            l_new, acc = l_cur, pv
        else:
            alpha = jnp.exp(m_old - m_new)
            l_new = alpha * l_s[b] + l_cur
            acc = alpha * acc_s[b] + pv
        if last:
            clat_s[b] = acc / l_new
        else:
            m_s[b] = m_new
            l_s[b] = l_new
            acc_s[b] = acc

    def compute_ctx(i0, i1):
        w32 = bwuv_v.bitcast(jnp.int32)
        for i in range(i0, i1):
            pair = _unpack_pair(w32[pl.ds(i, _DC, stride=_H // 2), :])
            for j in range(2):
                h = 2 * i + j
                r0 = clat_s[0, pl.ds(h, 1), :]
                r1 = clat_s[1, pl.ds(h, 1), :]
                lhs = jnp.where(row8 == 0, r0, jnp.where(row8 == 1, r1, 0.0))
                ctx_s[h] = _dot(lhs.astype(_bf16), pair[j])

    row8h = jax.lax.broadcasted_iota(jnp.int32, (8, _DH), 0)

    def a_head(i, slot):
        b = i % 2
        h = i // 2
        q8 = qa_s[h].astype(_bf16)
        s = _dot_t(q8, kv_buf[slot, 0])
        m = jnp.max(s, axis=-1, keepdims=True)
        p = jnp.exp(s - m)
        l = jnp.sum(p, axis=-1, keepdims=True)
        o = _dot(p.astype(_bf16), kv_buf[slot, 1]) / l
        o_s[h] = jnp.where(row8h == b, o, o_s[h])

    def out_proj(src_s, w_v, h0, h1):
        acc = None
        for h in range(h0, h1):
            t = _dot(src_s[h].astype(_bf16), w_v[pl.ds(h * _DH, _DH), :])
            acc = t if acc is None else acc + t
        return acc

    cx = pltpu.make_async_copy(x_hbm, x_ref, x_sem.at[0])
    cg = pltpu.make_async_copy(gw_hbm, gw_ref, x_sem.at[1])
    cx.start()
    cg.start()
    issue(u_w1)
    o_s[...] = jnp.zeros_like(o_s)
    cx.wait()
    cg.wait()
    x8f = load_x8()
    x8 = x8f.astype(_bf16)
    gate = jax.nn.sigmoid(jnp.sum(x8f * gw_ref[...].astype(_f32).reshape(1, _D), axis=-1, keepdims=True))

    issue(u_w2, 0, 64)
    wait_all(wq_v, w_sem.at[S_WQ])
    compute_qa(x8)
    issue(u_w2, 64, 128)
    wait_all(bwq_v, w_sem.at[S_BWQ])
    compute_qb(x8, 0, 8)
    issue(u_w2, 128, 192)
    compute_qb(x8, 8, 16)
    issue(u_w2, 192, 256)

    ck = [u_ckv(c) for c in range(NCK)]
    half = len(ck[0]) // 2
    issue(ck[0])
    wait_all(bwuk_v, w_sem.at[S_BWUK])
    compute_qlat(0, 8)
    issue(ck[1])
    compute_qlat(8, 16)

    kv0 = u_kv(0, 0)
    nkv = len(kv0)
    for c in range(NCK):
        for b in range(_B):
            if c + 2 < NCK:
                issue(ck[c + 2], b * half, (b + 1) * half)
            else:
                t = (c + 2 - NCK) * _B + b
                issue(kv0, t * nkv // 4, (t + 1) * nkv // 4)
            wait_all(ckv_v.at[b * NCK + c], w_sem.at[S_CKV + b * NCK + c])
            b_chunk(b, c)

    nbh = _B * _H

    def step(i, s, extra=None):
        issue(u_kv(i + 1, (s + 1) % _NSLOT))
        wait_all(kv_buf.at[s], kv_sem.at[s])
        a_head(i, s)
        if extra is not None:
            extra()

    NPEEL = _NPEEL
    wait_all(bwuv_v, w_sem.at[S_BWUV])
    for i in range(NPEEL):
        step(i, i % _NSLOT, functools.partial(compute_ctx, i * 16 // NPEEL, (i + 1) * 16 // NPEEL))

    def body(it, carry):
        for s in range(_NSLOT):
            step(it * _NSLOT + s, s)
        return carry

    NE = len(_END)
    ue = [u_end(e) for e in range(NE)]
    n_main = (nbh - 1) // _NSLOT
    jax.lax.fori_loop(NPEEL // _NSLOT, n_main, body, 0)
    for i in range(n_main * _NSLOT, nbh):
        s = i % _NSLOT
        if i + 1 < nbh:
            issue(u_kv(i + 1, (i + 1) % _NSLOT))
        else:
            issue(ue[0])
        wait_all(kv_buf.at[s], kv_sem.at[s])
        a_head(i, s)

    out_a = None
    out_b = None
    nxt = 1
    for e in range(NE):
        while nxt < min(e + 1 + _AHEAD[e], NE):
            issue(ue[nxt])
            nxt += 1
        h0, h1 = end_h[e], end_h[e + 1]
        wait_all(wo_v.at[pl.ds(h0 * _DH, (h1 - h0) * _DH)], w_sem.at[S_END + e])
        wait_all(bwo_v.at[pl.ds(h0 * _DH, (h1 - h0) * _DH)], w_sem.at[S_END + e])
        ta = out_proj(o_s, wo_v, h0, h1)
        tb = out_proj(ctx_s, bwo_v, h0, h1)
        out_a = ta if out_a is None else out_a + ta
        out_b = tb if out_b is None else out_b + tb
    res = gate * out_a + (1.0 - gate) * out_b
    out_ref[...] = res[0:2, :].astype(_bf16)


@jax.jit
def pallas_gated_mix__mha_block_cached__compressed_kv_cla__decode_kernel(
    A_x: jax.Array,
    A_k_cache: jax.Array,
    A_v_cache: jax.Array,
    A_wq: jax.Array,
    A_wo: jax.Array,
    B_x: jax.Array,
    B_c_kv: jax.Array,
    B_w_q: jax.Array,
    B_w_uk: jax.Array,
    B_w_uv: jax.Array,
    B_w_o: jax.Array,
    gate_w: jax.Array,
):
    del B_x
    k3 = A_k_cache.reshape(_B * _H, _SK, _DH)
    v3 = A_v_cache.reshape(_B * _H, _SK, _DH)
    ckv = B_c_kv.reshape(_B * _SK, _DC)
    bwq = B_w_q.reshape(_D * _H, _DH)
    bwuk = B_w_uk.reshape(_DC * _H, _DH)
    bwuv = B_w_uv.reshape(_DC * _H, _DH)
    bwo = B_w_o.reshape(_H * _DH, _D)
    x2 = A_x.reshape(_B, _D)

    hbm = pl.BlockSpec(memory_space=pl.ANY)
    vmem = pl.BlockSpec(memory_space=pltpu.VMEM)
    V = pltpu.VMEM
    scratch = [
        V((_NSLOT, 2, _SK, _DH), _bf16),
        V((_D, _H * _DH), _bf16),
        V((_H * _DH, _D), _bf16),
        V((_B * _NCK, _SK // _NCK, _DC), _bf16),
        V((_D * _H, _DH), _bf16),
        V((_DC * _H, _DH), _bf16),
        V((_DC * _H, _DH), _bf16),
        V((_H * _DH, _D), _bf16),
        V((_H, 8, _DH), _f32),
        V((_H, 8, _DH), _f32),
        V((_B, _H, _DC), _f32),
        V((_B, _H, _DC), _f32),
        V((_H, 8, _DH), _f32),
        V((_H, 8, _DH), _f32),
        V((_B, _H, 1), _f32),
        V((_B, _H, 1), _f32),
        V((_B, _H, _DC), _f32),
        V((_B, _D), _bf16),
        V((_D,), _bf16),
        pltpu.SemaphoreType.DMA((_NSLOT,)),
        pltpu.SemaphoreType.DMA((4 + 2 * _NCK + len(_END),)),
        pltpu.SemaphoreType.DMA((2,)),
    ]
    out = pl.pallas_call(
        _kernel,
        out_shape=jax.ShapeDtypeStruct((_B, _D), _bf16),
        in_specs=[hbm] * 11,
        out_specs=vmem,
        scratch_shapes=scratch,
        compiler_params=pltpu.CompilerParams(vmem_limit_bytes=100 * 1024 * 1024),
    )(x2, gate_w, k3, v3, A_wq, A_wo, ckv, bwq, bwuk, bwuv, bwo)
    return out.reshape(_B, 1, _D)
```

```python
import functools

import jax
import jax.numpy as jnp
import jax.experimental.pallas as pl
import jax.experimental.pallas.tpu as pltpu

_B, _H, _SK, _DH, _D, _DC = 2, 32, 8192, 128, 512, 512

_PIECE_ROWS = 128
_PRIO_KV, _RUN_KV = (0, 1), 1
_ROT_KV = 2
_ROT_W = 2
_ROT_C = 2
_ROT_E = 2
_PRIO_W, _RUN_W = (0, 1), 1
_PRIO_C, _RUN_C = (0, 1), 1
_PRIO_E, _RUN_E = (0, 1), 1
_CPU = 2
_LAG_C = 6
_NCK = 8
_END = (16, 8, 4, 2, 2)
_AHEAD = (1, 9, 9, 9, 9)
_NPEEL = 4
_NSLOT = 2

_f32 = jnp.float32
_bf16 = jnp.bfloat16


def _dot(a, b):
    return jnp.dot(a, b, preferred_element_type=_f32)


def _dot_t(a, b):
    return jax.lax.dot_general(a, b, (((1,), (1,)), ((), ())), preferred_element_type=_f32)


def _unpack_pair(blk):
    lo = pltpu.bitcast(blk << 16, _f32).astype(_bf16)
    hi = pltpu.bitcast(blk & jnp.int32(-65536), _f32).astype(_bf16)
    return lo, hi


def _kernel(x_hbm, gw_hbm,
            k_hbm, v_hbm, wq_hbm, wo_hbm, ckv_hbm, bwq_hbm, bwuk_hbm, bwuv_hbm, bwo_hbm,
            out_ref,
            kv_buf, wq_v, wo_v, ckv_v, bwq_v, bwuk_v, bwuv_v, bwo_v,
            qa_s, qb_s, qlat_s, clat_s, o_s, ctx_s, m_s, l_s, acc_s,
            x_ref, gw_ref, kv_sem, w_sem, x_sem):

    def rows(src, dst, nrow, n, sem, soff=0, doff=0):
        return [(src.at[pl.ds(soff + p * nrow, nrow)], dst.at[pl.ds(doff + p * nrow, nrow)], sem)
                for p in range(n)]

    def rot(u, mode):
        n = len(u)
        if mode == 0:
            return u
        if n % 64 == 0:
            if mode == 2:
                return [u[(p // 64) * 64 + (p % 4) * 16 + (p % 64) // 4] for p in range(n)]
            return [u[(p // 64) * 64 + (p % 2) * 32 + (p % 64) // 2] for p in range(n)]
        if n % 32 == 0:
            return [u[(p // 32) * 32 + (p % 2) * 16 + (p % 32) // 2] for p in range(n)]
        return u

    def zip2(u, v, run=_RUN_W, prio=_PRIO_W, mode=_ROT_W):
        u, v = rot(u, mode), rot(v, mode)
        out = []
        for j in range(0, len(u), run):
            out += u[j:j + run] + v[j:j + run]
        return [(a, b, c, prio[p % len(prio)]) for p, (a, b, c) in enumerate(out)]

    def issue(unit, lo=0, hi=None):
        for p in range(lo, len(unit) if hi is None else hi):
            src, dst, sem, prio = unit[p]
            pltpu.make_async_copy(src, dst, sem).start(priority=prio)

    def wait_all(dst, sem):
        pltpu.make_async_copy(dst, dst, sem).wait()

    S_WQ, S_BWQ, S_BWUK, S_BWUV = 0, 1, 2, 3
    S_CKV = 4
    NCK = _NCK
    CK = _SK // NCK
    S_END = S_CKV + 2 * NCK

    u_wq = [(wq_hbm.at[pl.ds((p // 4) * 16, 16), pl.ds((p % 4) * 1024, 1024)],
             wq_v.at[pl.ds((p // 4) * 16, 16), pl.ds((p % 4) * 1024, 1024)], w_sem.at[S_WQ])
            for p in range(128)]
    u_w1 = zip2(u_wq, rows(bwq_hbm, bwq_v, 128, 128, w_sem.at[S_BWQ]))
    u_w2 = zip2(rows(bwuk_hbm, bwuk_v, 128, 128, w_sem.at[S_BWUK]),
                rows(bwuv_hbm, bwuv_v, 128, 128, w_sem.at[S_BWUV]))

    CPU = _CPU

    def u_ckv(u):
        streams = []
        for b in range(_B):
            st = []
            for c in range(u * CPU, (u + 1) * CPU):
                st += rows(ckv_hbm, ckv_v.at[b * NCK + c], 32, CK // 32, w_sem.at[S_CKV + u], soff=b * _SK + c * CK)
            streams.append(st)
        return zip2(*streams, run=_RUN_C, prio=_PRIO_C, mode=_ROT_C)

    end_h = [0]
    for n in _END:
        end_h.append(end_h[-1] + n)

    def u_end(e):
        h0, n = end_h[e], _END[e]
        return zip2(*[rows(src, dst, 32, n * _DH // 32, w_sem.at[S_END + e], soff=h0 * _DH, doff=h0 * _DH)
                      for src, dst in ((wo_hbm, wo_v), (bwo_hbm, bwo_v))], run=_RUN_E, prio=_PRIO_E, mode=_ROT_E)

    def u_kv(i, slot):
        bh = (i % 2) * _H + i // 2
        n = _SK // _PIECE_ROWS
        return zip2(*[[(src.at[bh, pl.ds(p * _PIECE_ROWS, _PIECE_ROWS)],
                        kv_buf.at[slot, j, pl.ds(p * _PIECE_ROWS, _PIECE_ROWS)], kv_sem.at[slot])
                       for p in range(n)] for j, src in enumerate((k_hbm, v_hbm))], run=_RUN_KV, prio=_PRIO_KV, mode=_ROT_KV)

    row8 = jax.lax.broadcasted_iota(jnp.int32, (8, _D), 0)
    scale_a = _DH ** -0.5
    scale_b = _DH ** -0.5

    def load_x8():
        xf = x_ref[...].astype(_f32)
        x0 = xf[0:1]
        x1 = xf[1:2]
        return jnp.where(row8 == 0, x0, jnp.where(row8 == 1, x1, 0.0))

    def compute_qa(x8):
        q = _dot(x8, wq_v[...]) * scale_a
        for h in range(_H):
            qa_s[h] = q[:, h * _DH:(h + 1) * _DH]

    def compute_qb(x8, i0, i1):
        w32 = bwq_v.bitcast(jnp.int32)
        for i in range(i0, i1):
            lo, hi = _unpack_pair(w32[pl.ds(i, _D, stride=_H // 2), :])
            qb_s[2 * i] = _dot(x8, lo)
            qb_s[2 * i + 1] = _dot(x8, hi)

    def compute_qlat(i0, i1):
        w32 = bwuk_v.bitcast(jnp.int32)
        for i in range(i0, i1):
            pair = _unpack_pair(w32[pl.ds(i, _DC, stride=_H // 2), :])
            for j in range(2):
                h = 2 * i + j
                ql = _dot_t(qb_s[h].astype(_bf16), pair[j]) * scale_b
                qlat_s[0, pl.ds(h, 1), :] = ql[0:1, :]
                qlat_s[1, pl.ds(h, 1), :] = ql[1:2, :]

    def b_chunk(b, c):
        first = c == 0
        last = c == NCK - 1
        ck = ckv_v[b * NCK + c]
        s = _dot_t(qlat_s[b].astype(_bf16), ck)
        m_cur = jnp.max(s, axis=-1, keepdims=True)
        if first:
            m_new = m_cur
        else:
            m_old = m_s[b]
            m_new = jnp.maximum(m_old, m_cur)
        p = jnp.exp(s - m_new)
        l_cur = jnp.sum(p, axis=-1, keepdims=True)
        pv = _dot(p.astype(_bf16), ck)
        if first:
            l_new, acc = l_cur, pv
        else:
            alpha = jnp.exp(m_old - m_new)
            l_new = alpha * l_s[b] + l_cur
            acc = alpha * acc_s[b] + pv
        if last:
            clat_s[b] = acc / l_new
        else:
            m_s[b] = m_new
            l_s[b] = l_new
            acc_s[b] = acc

    def compute_ctx(i0, i1):
        w32 = bwuv_v.bitcast(jnp.int32)
        for i in range(i0, i1):
            pair = _unpack_pair(w32[pl.ds(i, _DC, stride=_H // 2), :])
            for j in range(2):
                h = 2 * i + j
                r0 = clat_s[0, pl.ds(h, 1), :]
                r1 = clat_s[1, pl.ds(h, 1), :]
                lhs = jnp.where(row8 == 0, r0, jnp.where(row8 == 1, r1, 0.0))
                ctx_s[h] = _dot(lhs.astype(_bf16), pair[j])

    row8h = jax.lax.broadcasted_iota(jnp.int32, (8, _DH), 0)

    def a_head(i, slot):
        b = i % 2
        h = i // 2
        q8 = qa_s[h].astype(_bf16)
        s = _dot_t(q8, kv_buf[slot, 0])
        m = jnp.max(s, axis=-1, keepdims=True)
        p = jnp.exp(s - m)
        l = jnp.sum(p, axis=-1, keepdims=True)
        o = _dot(p.astype(_bf16), kv_buf[slot, 1]) / l
        o_s[h] = jnp.where(row8h == b, o, o_s[h])

    def out_proj(src_s, w_v, h0, h1):
        acc = None
        for h in range(h0, h1):
            t = _dot(src_s[h].astype(_bf16), w_v[pl.ds(h * _DH, _DH), :])
            acc = t if acc is None else acc + t
        return acc

    cx = pltpu.make_async_copy(x_hbm, x_ref, x_sem.at[0])
    cg = pltpu.make_async_copy(gw_hbm, gw_ref, x_sem.at[1])
    cx.start()
    cg.start()
    issue(u_w1)
    o_s[...] = jnp.zeros_like(o_s)
    cx.wait()
    cg.wait()
    x8f = load_x8()
    x8 = x8f.astype(_bf16)
    gate = jax.nn.sigmoid(jnp.sum(x8f * gw_ref[...].astype(_f32).reshape(1, _D), axis=-1, keepdims=True))

    issue(u_w2, 0, 64)
    wait_all(wq_v, w_sem.at[S_WQ])
    compute_qa(x8)
    issue(u_w2, 64, 128)
    wait_all(bwq_v, w_sem.at[S_BWQ])
    compute_qb(x8, 0, 8)
    issue(u_w2, 128, 192)
    compute_qb(x8, 8, 16)
    issue(u_w2, 192, 256)

    NU = NCK // CPU
    stream = []
    for u in range(NU):
        stream += u_ckv(u)
    stream += u_kv(0, 0)
    SL = CK // 32
    LAG = _LAG_C
    pos = 0

    def issue_slices(upto):
        nonlocal pos
        hi = min(upto * SL, len(stream))
        if hi > pos:
            issue(stream, pos, hi)
            pos = hi

    issue_slices(1)
    wait_all(bwuk_v, w_sem.at[S_BWUK])
    compute_qlat(0, 8)
    issue_slices(2)
    compute_qlat(8, 16)

    t = 0
    for u in range(NU):
        for cc in range(CPU):
            for b in range(_B):
                issue_slices(t + LAG)
                if cc == 0 and b == 0:
                    for bb in range(_B):
                        wait_all(ckv_v.at[pl.ds(bb * NCK + u * CPU, CPU)], w_sem.at[S_CKV + u])
                b_chunk(b, u * CPU + cc)
                t += 1
    issue_slices(10 ** 6)

    nbh = _B * _H

    def step(i, s, extra=None):
        issue(u_kv(i + 1, (s + 1) % _NSLOT))
        wait_all(kv_buf.at[s], kv_sem.at[s])
        a_head(i, s)
        if extra is not None:
            extra()

    NPEEL = _NPEEL
    wait_all(bwuv_v, w_sem.at[S_BWUV])
    for i in range(NPEEL):
        step(i, i % _NSLOT, functools.partial(compute_ctx, i * 16 // NPEEL, (i + 1) * 16 // NPEEL))

    def body(it, carry):
        for s in range(_NSLOT):
            step(it * _NSLOT + s, s)
        return carry

    NE = len(_END)
    ue = [u_end(e) for e in range(NE)]
    n_main = (nbh - 1) // _NSLOT
    jax.lax.fori_loop(NPEEL // _NSLOT, n_main, body, 0)
    for i in range(n_main * _NSLOT, nbh):
        s = i % _NSLOT
        if i + 1 < nbh:
            issue(u_kv(i + 1, (i + 1) % _NSLOT))
        else:
            issue(ue[0])
        wait_all(kv_buf.at[s], kv_sem.at[s])
        a_head(i, s)

    out_a = None
    out_b = None
    nxt = 1
    for e in range(NE):
        while nxt < min(e + 1 + _AHEAD[e], NE):
            issue(ue[nxt])
            nxt += 1
        h0, h1 = end_h[e], end_h[e + 1]
        wait_all(wo_v.at[pl.ds(h0 * _DH, (h1 - h0) * _DH)], w_sem.at[S_END + e])
        wait_all(bwo_v.at[pl.ds(h0 * _DH, (h1 - h0) * _DH)], w_sem.at[S_END + e])
        ta = out_proj(o_s, wo_v, h0, h1)
        tb = out_proj(ctx_s, bwo_v, h0, h1)
        out_a = ta if out_a is None else out_a + ta
        out_b = tb if out_b is None else out_b + tb
    res = gate * out_a + (1.0 - gate) * out_b
    out_ref[...] = res[0:2, :].astype(_bf16)


@jax.jit
def pallas_gated_mix__mha_block_cached__compressed_kv_cla__decode_kernel(
    A_x: jax.Array,
    A_k_cache: jax.Array,
    A_v_cache: jax.Array,
    A_wq: jax.Array,
    A_wo: jax.Array,
    B_x: jax.Array,
    B_c_kv: jax.Array,
    B_w_q: jax.Array,
    B_w_uk: jax.Array,
    B_w_uv: jax.Array,
    B_w_o: jax.Array,
    gate_w: jax.Array,
):
    del B_x
    k3 = A_k_cache.reshape(_B * _H, _SK, _DH)
    v3 = A_v_cache.reshape(_B * _H, _SK, _DH)
    ckv = B_c_kv.reshape(_B * _SK, _DC)
    bwq = B_w_q.reshape(_D * _H, _DH)
    bwuk = B_w_uk.reshape(_DC * _H, _DH)
    bwuv = B_w_uv.reshape(_DC * _H, _DH)
    bwo = B_w_o.reshape(_H * _DH, _D)
    x2 = A_x.reshape(_B, _D)

    hbm = pl.BlockSpec(memory_space=pl.ANY)
    vmem = pl.BlockSpec(memory_space=pltpu.VMEM)
    V = pltpu.VMEM
    scratch = [
        V((_NSLOT, 2, _SK, _DH), _bf16),
        V((_D, _H * _DH), _bf16),
        V((_H * _DH, _D), _bf16),
        V((_B * _NCK, _SK // _NCK, _DC), _bf16),
        V((_D * _H, _DH), _bf16),
        V((_DC * _H, _DH), _bf16),
        V((_DC * _H, _DH), _bf16),
        V((_H * _DH, _D), _bf16),
        V((_H, 8, _DH), _f32),
        V((_H, 8, _DH), _f32),
        V((_B, _H, _DC), _f32),
        V((_B, _H, _DC), _f32),
        V((_H, 8, _DH), _f32),
        V((_H, 8, _DH), _f32),
        V((_B, _H, 1), _f32),
        V((_B, _H, 1), _f32),
        V((_B, _H, _DC), _f32),
        V((_B, _D), _bf16),
        V((_D,), _bf16),
        pltpu.SemaphoreType.DMA((_NSLOT,)),
        pltpu.SemaphoreType.DMA((4 + 2 * _NCK + len(_END),)),
        pltpu.SemaphoreType.DMA((2,)),
    ]
    out = pl.pallas_call(
        _kernel,
        out_shape=jax.ShapeDtypeStruct((_B, _D), _bf16),
        in_specs=[hbm] * 11,
        out_specs=vmem,
        scratch_shapes=scratch,
        compiler_params=pltpu.CompilerParams(vmem_limit_bytes=100 * 1024 * 1024),
    )(x2, gate_w, k3, v3, A_wq, A_wo, ckv, bwq, bwuk, bwuv, bwo)
    return out.reshape(_B, 1, _D)
```

```python
import functools

import jax
import jax.numpy as jnp
import jax.experimental.pallas as pl
import jax.experimental.pallas.tpu as pltpu

_B, _H, _SK, _DH, _D, _DC = 2, 32, 8192, 128, 512, 512

_PIECE_ROWS = 128
_PRIO_KV, _RUN_KV = (0, 1), 1
_ROT_KV = 2
_ROT_W = 2
_ROT_C = 2
_ROT_E = 2
_PRIO_W, _RUN_W = (0, 1), 1
_PRIO_C, _RUN_C = (0, 1), 1
_PRIO_E, _RUN_E = (0, 1), 1
_CPU = 2
_LAG_C = 6
_NCK = 8
_END = (16, 8, 4, 2, 2)
_AHEAD = (1, 9, 9, 9, 9)
_NPEEL = 4
_NSLOT = 2

_f32 = jnp.float32
_bf16 = jnp.bfloat16


def _dot(a, b):
    return jnp.dot(a, b, preferred_element_type=_f32)


def _dot_t(a, b):
    return jax.lax.dot_general(a, b, (((1,), (1,)), ((), ())), preferred_element_type=_f32)


def _unpack_pair(blk):
    lo = pltpu.bitcast(blk << 16, _f32).astype(_bf16)
    hi = pltpu.bitcast(blk & jnp.int32(-65536), _f32).astype(_bf16)
    return lo, hi


def _kernel(x_hbm, gw_hbm,
            k_hbm, v_hbm, wq_hbm, wo_hbm, ckv_hbm, bwq_hbm, bwuk_hbm, bwuv_hbm, bwo_hbm,
            out_ref,
            kv_buf, wq_v, wob_v, ckv_v, bwq_v, bwuk_v, bwuv_v,
            qa_s, qb_s, qlat_s, clat_s, o_s, ctx_s, m_s, l_s, acc_s,
            x_ref, gw_ref, kv_sem, w_sem, x_sem):

    def rows(src, dst, nrow, n, sem, soff=0, doff=0):
        return [(src.at[pl.ds(soff + p * nrow, nrow)], dst.at[pl.ds(doff + p * nrow, nrow)], sem)
                for p in range(n)]

    def rot(u, mode):
        n = len(u)
        if mode == 0:
            return u
        if n % 64 == 0:
            if mode == 2:
                return [u[(p // 64) * 64 + (p % 4) * 16 + (p % 64) // 4] for p in range(n)]
            return [u[(p // 64) * 64 + (p % 2) * 32 + (p % 64) // 2] for p in range(n)]
        if n % 32 == 0:
            return [u[(p // 32) * 32 + (p % 2) * 16 + (p % 32) // 2] for p in range(n)]
        return u

    def zip2(u, v, run=_RUN_W, prio=_PRIO_W, mode=_ROT_W):
        u, v = rot(u, mode), rot(v, mode)
        out = []
        for j in range(0, len(u), run):
            out += u[j:j + run] + v[j:j + run]
        return [(a, b, c, prio[p % len(prio)]) for p, (a, b, c) in enumerate(out)]

    def issue(unit, lo=0, hi=None):
        for p in range(lo, len(unit) if hi is None else hi):
            src, dst, sem, prio = unit[p]
            pltpu.make_async_copy(src, dst, sem).start(priority=prio)

    def wait_all(dst, sem):
        pltpu.make_async_copy(dst, dst, sem).wait()

    S_WQ, S_BWQ, S_BWUK, S_BWUV = 0, 1, 2, 3
    S_CKV = 4
    NCK = _NCK
    CK = _SK // NCK
    S_END = S_CKV + 2 * NCK

    u_wq = [(wq_hbm.at[pl.ds((p // 4) * 16, 16), pl.ds((p % 4) * 1024, 1024)],
             wq_v.at[pl.ds((p // 4) * 16, 16), pl.ds((p % 4) * 1024, 1024)], w_sem.at[S_WQ])
            for p in range(128)]
    u_w1 = zip2(u_wq, rows(bwq_hbm, bwq_v, 128, 128, w_sem.at[S_BWQ]))
    u_w2 = zip2(rows(bwuk_hbm, bwuk_v, 128, 128, w_sem.at[S_BWUK]),
                rows(bwuv_hbm, bwuv_v, 128, 128, w_sem.at[S_BWUV]))

    CPU = _CPU

    def u_ckv(u):
        streams = []
        for b in range(_B):
            st = []
            for c in range(u * CPU, (u + 1) * CPU):
                st += rows(ckv_hbm, ckv_v.at[u, b, c % CPU], 32, CK // 32, w_sem.at[S_CKV + u], soff=b * _SK + c * CK)
            streams.append(st)
        return zip2(*streams, run=_RUN_C, prio=_PRIO_C, mode=_ROT_C)

    end_h = [0]
    for n in _END:
        end_h.append(end_h[-1] + n)

    def u_end(e):
        h0, n = end_h[e], _END[e]
        return zip2(*[rows(src, wob_v.at[j], 32, n * _DH // 32, w_sem.at[S_END + e], soff=h0 * _DH, doff=h0 * _DH)
                      for j, src in enumerate((wo_hbm, bwo_hbm))], run=_RUN_E, prio=_PRIO_E, mode=_ROT_E)

    def u_kv(i, slot):
        bh = (i % 2) * _H + i // 2
        n = _SK // _PIECE_ROWS
        return zip2(*[[(src.at[bh, pl.ds(p * _PIECE_ROWS, _PIECE_ROWS)],
                        kv_buf.at[slot, j, pl.ds(p * _PIECE_ROWS, _PIECE_ROWS)], kv_sem.at[slot])
                       for p in range(n)] for j, src in enumerate((k_hbm, v_hbm))], run=_RUN_KV, prio=_PRIO_KV, mode=_ROT_KV)

    row8 = jax.lax.broadcasted_iota(jnp.int32, (8, _D), 0)
    scale_a = _DH ** -0.5
    scale_b = _DH ** -0.5

    def load_x8():
        xf = x_ref[...].astype(_f32)
        x0 = xf[0:1]
        x1 = xf[1:2]
        return jnp.where(row8 == 0, x0, jnp.where(row8 == 1, x1, 0.0))

    def compute_qa(x8):
        q = _dot(x8, wq_v[...]) * scale_a
        for h in range(_H):
            qa_s[h] = q[:, h * _DH:(h + 1) * _DH]

    def compute_qb(x8, i0, i1):
        w32 = bwq_v.bitcast(jnp.int32)
        for i in range(i0, i1):
            lo, hi = _unpack_pair(w32[pl.ds(i, _D, stride=_H // 2), :])
            qb_s[2 * i] = _dot(x8, lo)
            qb_s[2 * i + 1] = _dot(x8, hi)

    def compute_qlat(i0, i1):
        w32 = bwuk_v.bitcast(jnp.int32)
        for i in range(i0, i1):
            pair = _unpack_pair(w32[pl.ds(i, _DC, stride=_H // 2), :])
            for j in range(2):
                h = 2 * i + j
                ql = _dot_t(qb_s[h].astype(_bf16), pair[j]) * scale_b
                qlat_s[0, pl.ds(h, 1), :] = ql[0:1, :]
                qlat_s[1, pl.ds(h, 1), :] = ql[1:2, :]

    def b_chunk(b, c):
        first = c == 0
        last = c == NCK - 1
        ck = ckv_v[c // CPU, b, c % CPU]
        s = _dot_t(qlat_s[b].astype(_bf16), ck)
        m_cur = jnp.max(s, axis=-1, keepdims=True)
        if first:
            m_new = m_cur
        else:
            m_old = m_s[b]
            m_new = jnp.maximum(m_old, m_cur)
        p = jnp.exp(s - m_new)
        l_cur = jnp.sum(p, axis=-1, keepdims=True)
        pv = _dot(p.astype(_bf16), ck)
        if first:
            l_new, acc = l_cur, pv
        else:
            alpha = jnp.exp(m_old - m_new)
            l_new = alpha * l_s[b] + l_cur
            acc = alpha * acc_s[b] + pv
        if last:
            clat_s[b] = acc / l_new
        else:
            m_s[b] = m_new
            l_s[b] = l_new
            acc_s[b] = acc

    def compute_ctx(i0, i1):
        w32 = bwuv_v.bitcast(jnp.int32)
        for i in range(i0, i1):
            pair = _unpack_pair(w32[pl.ds(i, _DC, stride=_H // 2), :])
            for j in range(2):
                h = 2 * i + j
                r0 = clat_s[0, pl.ds(h, 1), :]
                r1 = clat_s[1, pl.ds(h, 1), :]
                lhs = jnp.where(row8 == 0, r0, jnp.where(row8 == 1, r1, 0.0))
                ctx_s[h] = _dot(lhs.astype(_bf16), pair[j])

    row8h = jax.lax.broadcasted_iota(jnp.int32, (8, _DH), 0)

    def a_head(i, slot):
        b = i % 2
        h = i // 2
        q8 = qa_s[h].astype(_bf16)
        s = _dot_t(q8, kv_buf[slot, 0])
        m = jnp.max(s, axis=-1, keepdims=True)
        p = jnp.exp(s - m)
        l = jnp.sum(p, axis=-1, keepdims=True)
        o = _dot(p.astype(_bf16), kv_buf[slot, 1]) / l
        o_s[h] = jnp.where(row8h == b, o, o_s[h])

    def out_proj(src_s, j, h0, h1):
        acc = None
        for h in range(h0, h1):
            t = _dot(src_s[h].astype(_bf16), wob_v[j, pl.ds(h * _DH, _DH), :])
            acc = t if acc is None else acc + t
        return acc

    cx = pltpu.make_async_copy(x_hbm, x_ref, x_sem.at[0])
    cg = pltpu.make_async_copy(gw_hbm, gw_ref, x_sem.at[1])
    cx.start()
    cg.start()
    issue(u_w1)
    o_s[...] = jnp.zeros_like(o_s)
    cx.wait()
    cg.wait()
    x8f = load_x8()
    x8 = x8f.astype(_bf16)
    gate = jax.nn.sigmoid(jnp.sum(x8f * gw_ref[...].astype(_f32).reshape(1, _D), axis=-1, keepdims=True))

    issue(u_w2, 0, 64)
    wait_all(wq_v, w_sem.at[S_WQ])
    compute_qa(x8)
    issue(u_w2, 64, 128)
    wait_all(bwq_v, w_sem.at[S_BWQ])
    compute_qb(x8, 0, 8)
    issue(u_w2, 128, 192)
    compute_qb(x8, 8, 16)
    issue(u_w2, 192, 256)

    NU = NCK // CPU
    stream = []
    for u in range(NU):
        stream += u_ckv(u)
    stream += u_kv(0, 0)
    SL = CK // 32
    LAG = _LAG_C
    pos = 0

    def issue_slices(upto):
        nonlocal pos
        hi = min(upto * SL, len(stream))
        if hi > pos:
            issue(stream, pos, hi)
            pos = hi

    issue_slices(1)
    wait_all(bwuk_v, w_sem.at[S_BWUK])
    compute_qlat(0, 8)
    issue_slices(2)
    compute_qlat(8, 16)

    t = 0
    for u in range(NU):
        for cc in range(CPU):
            for b in range(_B):
                issue_slices(t + LAG)
                if cc == 0 and b == 0:
                    wait_all(ckv_v.at[u], w_sem.at[S_CKV + u])
                b_chunk(b, u * CPU + cc)
                t += 1
    issue_slices(10 ** 6)

    nbh = _B * _H

    def step(i, s, extra=None):
        issue(u_kv(i + 1, (s + 1) % _NSLOT))
        wait_all(kv_buf.at[s], kv_sem.at[s])
        a_head(i, s)
        if extra is not None:
            extra()

    NPEEL = _NPEEL
    wait_all(bwuv_v, w_sem.at[S_BWUV])
    for i in range(NPEEL):
        step(i, i % _NSLOT, functools.partial(compute_ctx, i * 16 // NPEEL, (i + 1) * 16 // NPEEL))

    def body(it, carry):
        for s in range(_NSLOT):
            step(it * _NSLOT + s, s)
        return carry

    NE = len(_END)
    ue = [u_end(e) for e in range(NE)]
    n_main = (nbh - 1) // _NSLOT
    jax.lax.fori_loop(NPEEL // _NSLOT, n_main, body, 0)
    for i in range(n_main * _NSLOT, nbh):
        s = i % _NSLOT
        if i + 1 < nbh:
            issue(u_kv(i + 1, (i + 1) % _NSLOT))
        else:
            issue(ue[0])
        wait_all(kv_buf.at[s], kv_sem.at[s])
        a_head(i, s)

    out_a = None
    out_b = None
    nxt = 1
    for e in range(NE):
        while nxt < min(e + 1 + _AHEAD[e], NE):
            issue(ue[nxt])
            nxt += 1
        h0, h1 = end_h[e], end_h[e + 1]
        wait_all(wob_v.at[:, pl.ds(h0 * _DH, (h1 - h0) * _DH)], w_sem.at[S_END + e])
        ta = out_proj(o_s, 0, h0, h1)
        tb = out_proj(ctx_s, 1, h0, h1)
        out_a = ta if out_a is None else out_a + ta
        out_b = tb if out_b is None else out_b + tb
    res = gate * out_a + (1.0 - gate) * out_b
    out_ref[...] = res[0:2, :].astype(_bf16)


@jax.jit
def pallas_gated_mix__mha_block_cached__compressed_kv_cla__decode_kernel(
    A_x: jax.Array,
    A_k_cache: jax.Array,
    A_v_cache: jax.Array,
    A_wq: jax.Array,
    A_wo: jax.Array,
    B_x: jax.Array,
    B_c_kv: jax.Array,
    B_w_q: jax.Array,
    B_w_uk: jax.Array,
    B_w_uv: jax.Array,
    B_w_o: jax.Array,
    gate_w: jax.Array,
):
    del B_x
    k3 = A_k_cache.reshape(_B * _H, _SK, _DH)
    v3 = A_v_cache.reshape(_B * _H, _SK, _DH)
    ckv = B_c_kv.reshape(_B * _SK, _DC)
    bwq = B_w_q.reshape(_D * _H, _DH)
    bwuk = B_w_uk.reshape(_DC * _H, _DH)
    bwuv = B_w_uv.reshape(_DC * _H, _DH)
    bwo = B_w_o.reshape(_H * _DH, _D)
    x2 = A_x.reshape(_B, _D)

    hbm = pl.BlockSpec(memory_space=pl.ANY)
    vmem = pl.BlockSpec(memory_space=pltpu.VMEM)
    V = pltpu.VMEM
    scratch = [
        V((_NSLOT, 2, _SK, _DH), _bf16),
        V((_D, _H * _DH), _bf16),
        V((2, _H * _DH, _D), _bf16),
        V((_NCK // _CPU, _B, _CPU, _SK // _NCK, _DC), _bf16),
        V((_D * _H, _DH), _bf16),
        V((_DC * _H, _DH), _bf16),
        V((_DC * _H, _DH), _bf16),
        V((_H, 8, _DH), _f32),
        V((_H, 8, _DH), _f32),
        V((_B, _H, _DC), _f32),
        V((_B, _H, _DC), _f32),
        V((_H, 8, _DH), _f32),
        V((_H, 8, _DH), _f32),
        V((_B, _H, 1), _f32),
        V((_B, _H, 1), _f32),
        V((_B, _H, _DC), _f32),
        V((_B, _D), _bf16),
        V((_D,), _bf16),
        pltpu.SemaphoreType.DMA((_NSLOT,)),
        pltpu.SemaphoreType.DMA((4 + 2 * _NCK + len(_END),)),
        pltpu.SemaphoreType.DMA((2,)),
    ]
    out = pl.pallas_call(
        _kernel,
        out_shape=jax.ShapeDtypeStruct((_B, _D), _bf16),
        in_specs=[hbm] * 11,
        out_specs=vmem,
        scratch_shapes=scratch,
        compiler_params=pltpu.CompilerParams(vmem_limit_bytes=100 * 1024 * 1024),
    )(x2, gate_w, k3, v3, A_wq, A_wo, ckv, bwq, bwuk, bwuv, bwo)
    return out.reshape(_B, 1, _D)
```

```python
import functools

import jax
import jax.numpy as jnp
import jax.experimental.pallas as pl
import jax.experimental.pallas.tpu as pltpu

_B, _H, _SK, _DH, _D, _DC = 2, 32, 8192, 128, 512, 512

_PIECE_ROWS = 128
_VX_KV = 40
_NCK = 8
_CPU = 2
_LAG_C = 6
_END = (16, 8, 4, 2, 2)
_AHEAD = (1, 9, 9, 9, 9)
_NPEEL = 4
_NSLOT = 2

_f32 = jnp.float32
_bf16 = jnp.bfloat16


def _dot(a, b):
    return jnp.dot(a, b, preferred_element_type=_f32)


def _dot_t(a, b):
    return jax.lax.dot_general(a, b, (((1,), (1,)), ((), ())), preferred_element_type=_f32)


def _unpack_pair(blk):
    lo = pltpu.bitcast(blk << 16, _f32).astype(_bf16)
    hi = pltpu.bitcast(blk & jnp.int32(-65536), _f32).astype(_bf16)
    return lo, hi


def _kernel(x_hbm, gw_hbm,
            k_hbm, v_hbm, wq_hbm, wo_hbm, ckv_hbm, bwq_hbm, bwuk_hbm, bwuv_hbm, bwo_hbm,
            out_ref,
            kv_buf, wq_v, wob_v, ckv_v, bwq_v, bwuk_v, bwuv_v,
            qa_s, qb_s, qlat_s, clat_s, o_s, ctx_s, m_s, l_s, acc_s,
            x_ref, gw_ref, kv_sem, w_sem, x_sem):

    def rows(src, dst, nrow, n, sem, soff=0, doff=0):
        return [(src.at[pl.ds(soff + p * nrow, nrow)], dst.at[pl.ds(doff + p * nrow, nrow)], sem)
                for p in range(n)]

    def rot(u):
        n = len(u)
        if n % 64 == 0:
            return [u[(p // 64) * 64 + (p % 4) * 16 + (p % 64) // 4] for p in range(n)]
        if n % 32 == 0:
            return [u[(p // 32) * 32 + (p % 2) * 16 + (p % 32) // 2] for p in range(n)]
        return u

    def zip2(u, v, vx=0):
        v = [v[p ^ vx] for p in range(len(v))]
        out = []
        for a, b in zip(rot(u), rot(v)):
            out += [a + (0,), b + (1,)]
        return out

    def issue(unit, lo=0, hi=None):
        for p in range(lo, len(unit) if hi is None else hi):
            src, dst, sem, prio = unit[p]
            pltpu.make_async_copy(src, dst, sem).start(priority=prio)

    def wait_all(dst, sem):
        pltpu.make_async_copy(dst, dst, sem).wait()

    NCK, CPU = _NCK, _CPU
    CK = _SK // NCK
    NU = NCK // CPU
    S_WQ, S_BWQ, S_BWUK, S_BWUV = 0, 1, 2, 3
    S_CKV = 4
    S_END = S_CKV + NU

    u_wq = [(wq_hbm.at[pl.ds((p // 2) * 8, 8), pl.ds((p % 2) * 2048, 2048)],
             wq_v.at[pl.ds((p // 2) * 8, 8), pl.ds((p % 2) * 2048, 2048)], w_sem.at[S_WQ])
            for p in range(128)]
    u_w1 = zip2(u_wq, rows(bwq_hbm, bwq_v, 128, 128, w_sem.at[S_BWQ]))
    u_w2 = zip2(rows(bwuk_hbm, bwuk_v, 128, 128, w_sem.at[S_BWUK]),
                rows(bwuv_hbm, bwuv_v, 128, 128, w_sem.at[S_BWUV]))

    def u_ckv(u):
        streams = []
        for b in range(_B):
            st = []
            for c in range(u * CPU, (u + 1) * CPU):
                st += rows(ckv_hbm, ckv_v.at[u, b, c % CPU], 32, CK // 32, w_sem.at[S_CKV + u],
                           soff=b * _SK + c * CK)
            streams.append(st)
        return zip2(*streams)

    end_h = [0]
    for n in _END:
        end_h.append(end_h[-1] + n)

    def u_end(e):
        h0, n = end_h[e], _END[e]
        return zip2(*[rows(src, wob_v.at[j], 32, n * _DH // 32, w_sem.at[S_END + e], soff=h0 * _DH, doff=h0 * _DH)
                      for j, src in enumerate((wo_hbm, bwo_hbm))])

    def u_kv(i, slot):
        bh = (i % 2) * _H + i // 2
        n = _SK // _PIECE_ROWS
        return zip2(*[[(src.at[bh, pl.ds(p * _PIECE_ROWS, _PIECE_ROWS)],
                        kv_buf.at[slot, j, pl.ds(p * _PIECE_ROWS, _PIECE_ROWS)], kv_sem.at[slot])
                       for p in range(n)] for j, src in enumerate((k_hbm, v_hbm))], vx=_VX_KV)

    row8 = jax.lax.broadcasted_iota(jnp.int32, (8, _D), 0)
    scale_a = _DH ** -0.5
    scale_b = _DH ** -0.5

    def load_x8():
        xf = x_ref[...].astype(_f32)
        x0 = xf[0:1]
        x1 = xf[1:2]
        return jnp.where(row8 == 0, x0, jnp.where(row8 == 1, x1, 0.0))

    def compute_qa(x8):
        q = _dot(x8, wq_v[...]) * scale_a
        for h in range(_H):
            qa_s[h] = q[:, h * _DH:(h + 1) * _DH]

    def compute_qb(x8, i0, i1):
        w32 = bwq_v.bitcast(jnp.int32)
        for i in range(i0, i1):
            lo, hi = _unpack_pair(w32[pl.ds(i, _D, stride=_H // 2), :])
            qb_s[2 * i] = _dot(x8, lo)
            qb_s[2 * i + 1] = _dot(x8, hi)

    def compute_qlat(i0, i1):
        w32 = bwuk_v.bitcast(jnp.int32)
        for i in range(i0, i1):
            pair = _unpack_pair(w32[pl.ds(i, _DC, stride=_H // 2), :])
            for j in range(2):
                h = 2 * i + j
                ql = _dot_t(qb_s[h].astype(_bf16), pair[j]) * scale_b
                qlat_s[0, pl.ds(h, 1), :] = ql[0:1, :]
                qlat_s[1, pl.ds(h, 1), :] = ql[1:2, :]

    def b_chunk(b, c):
        first = c == 0
        last = c == NCK - 1
        ck = ckv_v[c // CPU, b, c % CPU]
        s = _dot_t(qlat_s[b].astype(_bf16), ck)
        m_cur = jnp.max(s, axis=-1, keepdims=True)
        if first:
            m_new = m_cur
        else:
            m_old = m_s[b]
            m_new = jnp.maximum(m_old, m_cur)
        p = jnp.exp(s - m_new)
        l_cur = jnp.sum(p, axis=-1, keepdims=True)
        pv = _dot(p.astype(_bf16), ck)
        if first:
            l_new, acc = l_cur, pv
        else:
            alpha = jnp.exp(m_old - m_new)
            l_new = alpha * l_s[b] + l_cur
            acc = alpha * acc_s[b] + pv
        if last:
            clat_s[b] = acc / l_new
        else:
            m_s[b] = m_new
            l_s[b] = l_new
            acc_s[b] = acc

    def compute_ctx(i0, i1):
        w32 = bwuv_v.bitcast(jnp.int32)
        for i in range(i0, i1):
            pair = _unpack_pair(w32[pl.ds(i, _DC, stride=_H // 2), :])
            for j in range(2):
                h = 2 * i + j
                r0 = clat_s[0, pl.ds(h, 1), :]
                r1 = clat_s[1, pl.ds(h, 1), :]
                lhs = jnp.where(row8 == 0, r0, jnp.where(row8 == 1, r1, 0.0))
                ctx_s[h] = _dot(lhs.astype(_bf16), pair[j])

    row8h = jax.lax.broadcasted_iota(jnp.int32, (8, _DH), 0)

    def a_head(i, slot):
        b = i % 2
        h = i // 2
        q8 = qa_s[h].astype(_bf16)
        s = _dot_t(q8, kv_buf[slot, 0])
        m = jnp.max(s, axis=-1, keepdims=True)
        p = jnp.exp(s - m)
        l = jnp.sum(p, axis=-1, keepdims=True)
        o = _dot(p.astype(_bf16), kv_buf[slot, 1]) / l
        o_s[h] = jnp.where(row8h == b, o, o_s[h])

    def out_proj(src_s, j, h0, h1):
        acc = None
        for h in range(h0, h1):
            t = _dot(src_s[h].astype(_bf16), wob_v[j, pl.ds(h * _DH, _DH), :])
            acc = t if acc is None else acc + t
        return acc

    cx = pltpu.make_async_copy(x_hbm, x_ref, x_sem.at[0])
    cg = pltpu.make_async_copy(gw_hbm, gw_ref, x_sem.at[1])
    cx.start()
    cg.start()
    issue(u_w1)
    o_s[...] = jnp.zeros_like(o_s)
    cx.wait()
    cg.wait()
    x8f = load_x8()
    x8 = x8f.astype(_bf16)
    gate = jax.nn.sigmoid(jnp.sum(x8f * gw_ref[...].astype(_f32).reshape(1, _D), axis=-1, keepdims=True))

    issue(u_w2, 0, 64)
    wait_all(wq_v, w_sem.at[S_WQ])
    compute_qa(x8)
    issue(u_w2, 64, 128)
    wait_all(bwq_v, w_sem.at[S_BWQ])
    compute_qb(x8, 0, 8)
    issue(u_w2, 128, 192)
    compute_qb(x8, 8, 16)
    issue(u_w2, 192, 256)

    stream = []
    for u in range(NU):
        stream += u_ckv(u)
    stream += u_kv(0, 0)
    SL = CK // 32
    LAG = _LAG_C
    pos = 0

    def issue_slices(upto):
        nonlocal pos
        hi = min(upto * SL, len(stream))
        if hi > pos:
            issue(stream, pos, hi)
            pos = hi

    issue_slices(1)
    wait_all(bwuk_v, w_sem.at[S_BWUK])
    compute_qlat(0, 8)
    issue_slices(2)
    compute_qlat(8, 16)

    t = 0
    for u in range(NU):
        for cc in range(CPU):
            for b in range(_B):
                issue_slices(t + LAG)
                if cc == 0 and b == 0:
                    wait_all(ckv_v.at[u], w_sem.at[S_CKV + u])
                b_chunk(b, u * CPU + cc)
                t += 1
    issue_slices(10 ** 6)

    nbh = _B * _H

    def step(i, s, extra=None):
        issue(u_kv(i + 1, (s + 1) % _NSLOT))
        wait_all(kv_buf.at[s], kv_sem.at[s])
        a_head(i, s)
        if extra is not None:
            extra()

    NPEEL = _NPEEL
    wait_all(bwuv_v, w_sem.at[S_BWUV])
    for i in range(NPEEL):
        step(i, i % _NSLOT, functools.partial(compute_ctx, i * 16 // NPEEL, (i + 1) * 16 // NPEEL))

    def body(it, carry):
        for s in range(_NSLOT):
            step(it * _NSLOT + s, s)
        return carry

    NE = len(_END)
    ue = [u_end(e) for e in range(NE)]
    n_main = (nbh - 1) // _NSLOT
    jax.lax.fori_loop(NPEEL // _NSLOT, n_main, body, 0)
    for i in range(n_main * _NSLOT, nbh):
        s = i % _NSLOT
        if i + 1 < nbh:
            issue(u_kv(i + 1, (i + 1) % _NSLOT))
        else:
            issue(ue[0])
        wait_all(kv_buf.at[s], kv_sem.at[s])
        a_head(i, s)

    out_a = None
    out_b = None
    nxt = 1
    for e in range(NE):
        while nxt < min(e + 1 + _AHEAD[e], NE):
            issue(ue[nxt])
            nxt += 1
        h0, h1 = end_h[e], end_h[e + 1]
        wait_all(wob_v.at[:, pl.ds(h0 * _DH, (h1 - h0) * _DH)], w_sem.at[S_END + e])
        ta = out_proj(o_s, 0, h0, h1)
        tb = out_proj(ctx_s, 1, h0, h1)
        out_a = ta if out_a is None else out_a + ta
        out_b = tb if out_b is None else out_b + tb
    res = gate * out_a + (1.0 - gate) * out_b
    out_ref[...] = res[0:2, :].astype(_bf16)


@jax.jit
def pallas_gated_mix__mha_block_cached__compressed_kv_cla__decode_kernel(
    A_x: jax.Array,
    A_k_cache: jax.Array,
    A_v_cache: jax.Array,
    A_wq: jax.Array,
    A_wo: jax.Array,
    B_x: jax.Array,
    B_c_kv: jax.Array,
    B_w_q: jax.Array,
    B_w_uk: jax.Array,
    B_w_uv: jax.Array,
    B_w_o: jax.Array,
    gate_w: jax.Array,
):
    del B_x
    k3 = A_k_cache.reshape(_B * _H, _SK, _DH)
    v3 = A_v_cache.reshape(_B * _H, _SK, _DH)
    ckv = B_c_kv.reshape(_B * _SK, _DC)
    bwq = B_w_q.reshape(_D * _H, _DH)
    bwuk = B_w_uk.reshape(_DC * _H, _DH)
    bwuv = B_w_uv.reshape(_DC * _H, _DH)
    bwo = B_w_o.reshape(_H * _DH, _D)
    x2 = A_x.reshape(_B, _D)

    hbm = pl.BlockSpec(memory_space=pl.ANY)
    vmem = pl.BlockSpec(memory_space=pltpu.VMEM)
    V = pltpu.VMEM
    scratch = [
        V((_NSLOT, 2, _SK, _DH), _bf16),
        V((_D, _H * _DH), _bf16),
        V((2, _H * _DH, _D), _bf16),
        V((_NCK // _CPU, _B, _CPU, _SK // _NCK, _DC), _bf16),
        V((_D * _H, _DH), _bf16),
        V((_DC * _H, _DH), _bf16),
        V((_DC * _H, _DH), _bf16),
        V((_H, 8, _DH), _f32),
        V((_H, 8, _DH), _f32),
        V((_B, _H, _DC), _f32),
        V((_B, _H, _DC), _f32),
        V((_H, 8, _DH), _f32),
        V((_H, 8, _DH), _f32),
        V((_B, _H, 1), _f32),
        V((_B, _H, 1), _f32),
        V((_B, _H, _DC), _f32),
        V((_B, _D), _bf16),
        V((_D,), _bf16),
        pltpu.SemaphoreType.DMA((_NSLOT,)),
        pltpu.SemaphoreType.DMA((4 + _NCK // _CPU + len(_END),)),
        pltpu.SemaphoreType.DMA((2,)),
    ]
    out = pl.pallas_call(
        _kernel,
        out_shape=jax.ShapeDtypeStruct((_B, _D), _bf16),
        in_specs=[hbm] * 11,
        out_specs=vmem,
        scratch_shapes=scratch,
        compiler_params=pltpu.CompilerParams(vmem_limit_bytes=100 * 1024 * 1024),
    )(x2, gate_w, k3, v3, A_wq, A_wo, ckv, bwq, bwuk, bwuv, bwo)
    return out.reshape(_B, 1, _D)
```

```python
import functools

import jax
import jax.numpy as jnp
import jax.experimental.pallas as pl
import jax.experimental.pallas.tpu as pltpu

_B, _H, _SK, _DH, _D, _DC = 2, 32, 8192, 128, 512, 512

_PIECE_ROWS = 128
_VX_KV = 40
_NCK = 8
_CPU = 2
_LAG_C = 7
_END = (16, 8, 4, 2, 2)
_AHEAD = (1, 9, 9, 9, 9)
_NPEEL = 4
_NSLOT = 2

_f32 = jnp.float32
_bf16 = jnp.bfloat16


def _dot(a, b):
    return jnp.dot(a, b, preferred_element_type=_f32)


def _dot_t(a, b):
    return jax.lax.dot_general(a, b, (((1,), (1,)), ((), ())), preferred_element_type=_f32)


def _unpack_pair(blk):
    lo = pltpu.bitcast(blk << 16, _f32).astype(_bf16)
    hi = pltpu.bitcast(blk & jnp.int32(-65536), _f32).astype(_bf16)
    return lo, hi


def _kernel(x_hbm, gw_hbm,
            k_hbm, v_hbm, wq_hbm, wo_hbm, ckv_hbm, bwq_hbm, bwuk_hbm, bwuv_hbm, bwo_hbm,
            out_ref,
            kv_buf, wq_v, wob_v, ckv_v, bwq_v, bwuk_v, bwuv_v,
            qa_s, qb_s, qlat_s, clat_s, o_s, ctx_s, m_s, l_s, acc_s,
            x_ref, gw_ref, kv_sem, w_sem, x_sem):

    def rows(src, dst, nrow, n, sem, soff=0, doff=0):
        return [(src.at[pl.ds(soff + p * nrow, nrow)], dst.at[pl.ds(doff + p * nrow, nrow)], sem)
                for p in range(n)]

    def rot(u):
        n = len(u)
        if n % 64 == 0:
            return [u[(p // 64) * 64 + (p % 4) * 16 + (p % 64) // 4] for p in range(n)]
        if n % 32 == 0:
            return [u[(p // 32) * 32 + (p % 2) * 16 + (p % 32) // 2] for p in range(n)]
        return u

    def zip2(u, v, vx=0):
        v = [v[p ^ vx] for p in range(len(v))]
        out = []
        for a, b in zip(rot(u), rot(v)):
            out += [a + (0,), b + (1,)]
        return out

    def issue(unit, lo=0, hi=None):
        for p in range(lo, len(unit) if hi is None else hi):
            src, dst, sem, prio = unit[p]
            pltpu.make_async_copy(src, dst, sem).start(priority=prio)

    def wait_all(dst, sem):
        pltpu.make_async_copy(dst, dst, sem).wait()

    NCK, CPU = _NCK, _CPU
    CK = _SK // NCK
    NU = NCK // CPU
    S_WQ, S_BWQ, S_BWUK, S_BWUV = 0, 1, 2, 3
    S_CKV = 4
    S_END = S_CKV + NU

    u_wq = [(wq_hbm.at[pl.ds((p // 4) * 16, 16), pl.ds((p % 4) * 1024, 1024)],
             wq_v.at[pl.ds((p // 4) * 16, 16), pl.ds((p % 4) * 1024, 1024)], w_sem.at[S_WQ])
            for p in range(128)]
    u_w1 = zip2(u_wq, rows(bwq_hbm, bwq_v, 128, 128, w_sem.at[S_BWQ]))
    u_w2 = zip2(rows(bwuk_hbm, bwuk_v, 128, 128, w_sem.at[S_BWUK]),
                rows(bwuv_hbm, bwuv_v, 128, 128, w_sem.at[S_BWUV]))

    def u_ckv(u):
        streams = []
        for b in range(_B):
            st = []
            for c in range(u * CPU, (u + 1) * CPU):
                st += rows(ckv_hbm, ckv_v.at[u, b, c % CPU], 32, CK // 32, w_sem.at[S_CKV + u],
                           soff=b * _SK + c * CK)
            streams.append(st)
        return zip2(*streams)

    end_h = [0]
    for n in _END:
        end_h.append(end_h[-1] + n)

    def u_end(e):
        h0, n = end_h[e], _END[e]
        return zip2(*[rows(src, wob_v.at[j], 32, n * _DH // 32, w_sem.at[S_END + e], soff=h0 * _DH, doff=h0 * _DH)
                      for j, src in enumerate((wo_hbm, bwo_hbm))])

    def u_kv(i, slot):
        bh = (i % 2) * _H + i // 2
        n = _SK // _PIECE_ROWS
        return zip2(*[[(src.at[bh, pl.ds(p * _PIECE_ROWS, _PIECE_ROWS)],
                        kv_buf.at[slot, j, pl.ds(p * _PIECE_ROWS, _PIECE_ROWS)], kv_sem.at[slot])
                       for p in range(n)] for j, src in enumerate((k_hbm, v_hbm))], vx=_VX_KV)

    row8 = jax.lax.broadcasted_iota(jnp.int32, (8, _D), 0)
    scale_a = _DH ** -0.5
    scale_b = _DH ** -0.5

    def load_x8():
        xf = x_ref[...].astype(_f32)
        x0 = xf[0:1]
        x1 = xf[1:2]
        return jnp.where(row8 == 0, x0, jnp.where(row8 == 1, x1, 0.0))

    def compute_qa(x8):
        q = _dot(x8, wq_v[...]) * scale_a
        for h in range(_H):
            qa_s[h] = q[:, h * _DH:(h + 1) * _DH]

    def compute_qb(x8, i0, i1):
        w32 = bwq_v.bitcast(jnp.int32)
        for i in range(i0, i1):
            lo, hi = _unpack_pair(w32[pl.ds(i, _D, stride=_H // 2), :])
            qb_s[2 * i] = _dot(x8, lo)
            qb_s[2 * i + 1] = _dot(x8, hi)

    def compute_qlat(i0, i1):
        w32 = bwuk_v.bitcast(jnp.int32)
        for i in range(i0, i1):
            pair = _unpack_pair(w32[pl.ds(i, _DC, stride=_H // 2), :])
            for j in range(2):
                h = 2 * i + j
                ql = _dot_t(qb_s[h].astype(_bf16), pair[j]) * scale_b
                qlat_s[0, pl.ds(h, 1), :] = ql[0:1, :]
                qlat_s[1, pl.ds(h, 1), :] = ql[1:2, :]

    def b_chunk(b, c):
        first = c == 0
        last = c == NCK - 1
        ck = ckv_v[c // CPU, b, c % CPU]
        s = _dot_t(qlat_s[b].astype(_bf16), ck)
        m_cur = jnp.max(s, axis=-1, keepdims=True)
        if first:
            m_new = m_cur
        else:
            m_old = m_s[b]
            m_new = jnp.maximum(m_old, m_cur)
        p = jnp.exp(s - m_new)
        l_cur = jnp.sum(p, axis=-1, keepdims=True)
        pv = _dot(p.astype(_bf16), ck)
        if first:
            l_new, acc = l_cur, pv
        else:
            alpha = jnp.exp(m_old - m_new)
            l_new = alpha * l_s[b] + l_cur
            acc = alpha * acc_s[b] + pv
        if last:
            clat_s[b] = acc / l_new
        else:
            m_s[b] = m_new
            l_s[b] = l_new
            acc_s[b] = acc

    def compute_ctx(i0, i1):
        w32 = bwuv_v.bitcast(jnp.int32)
        for i in range(i0, i1):
            pair = _unpack_pair(w32[pl.ds(i, _DC, stride=_H // 2), :])
            for j in range(2):
                h = 2 * i + j
                r0 = clat_s[0, pl.ds(h, 1), :]
                r1 = clat_s[1, pl.ds(h, 1), :]
                lhs = jnp.where(row8 == 0, r0, jnp.where(row8 == 1, r1, 0.0))
                ctx_s[h] = _dot(lhs.astype(_bf16), pair[j])

    row8h = jax.lax.broadcasted_iota(jnp.int32, (8, _DH), 0)

    def a_head(i, slot):
        b = i % 2
        h = i // 2
        q8 = qa_s[h].astype(_bf16)
        s = _dot_t(q8, kv_buf[slot, 0])
        m = jnp.max(s, axis=-1, keepdims=True)
        p = jnp.exp(s - m)
        l = jnp.sum(p, axis=-1, keepdims=True)
        o = _dot(p.astype(_bf16), kv_buf[slot, 1]) / l
        o_s[h] = jnp.where(row8h == b, o, o_s[h])

    def out_proj(src_s, j, h0, h1):
        acc = None
        for h in range(h0, h1):
            t = _dot(src_s[h].astype(_bf16), wob_v[j, pl.ds(h * _DH, _DH), :])
            acc = t if acc is None else acc + t
        return acc

    cx = pltpu.make_async_copy(x_hbm, x_ref, x_sem.at[0])
    cg = pltpu.make_async_copy(gw_hbm, gw_ref, x_sem.at[1])
    cx.start()
    cg.start()
    issue(u_w1)
    o_s[...] = jnp.zeros_like(o_s)
    cx.wait()
    cg.wait()
    x8f = load_x8()
    x8 = x8f.astype(_bf16)
    gate = jax.nn.sigmoid(jnp.sum(x8f * gw_ref[...].astype(_f32).reshape(1, _D), axis=-1, keepdims=True))

    issue(u_w2, 0, 64)
    wait_all(wq_v, w_sem.at[S_WQ])
    compute_qa(x8)
    issue(u_w2, 64, 128)
    wait_all(bwq_v, w_sem.at[S_BWQ])
    compute_qb(x8, 0, 8)
    issue(u_w2, 128, 192)
    compute_qb(x8, 8, 16)
    issue(u_w2, 192, 256)

    stream = []
    for u in range(NU):
        stream += u_ckv(u)
    stream += u_kv(0, 0) + u_kv(1, 1)
    SL = CK // 32
    LAG = _LAG_C
    pos = 0

    def issue_slices(upto):
        nonlocal pos
        hi = min(upto * SL, len(stream))
        if hi > pos:
            issue(stream, pos, hi)
            pos = hi

    issue_slices(1)
    wait_all(bwuk_v, w_sem.at[S_BWUK])
    compute_qlat(0, 8)
    issue_slices(2)
    compute_qlat(8, 16)

    t = 0
    for u in range(NU):
        for cc in range(CPU):
            for b in range(_B):
                issue_slices(t + LAG)
                if cc == 0 and b == 0:
                    wait_all(ckv_v.at[u], w_sem.at[S_CKV + u])
                b_chunk(b, u * CPU + cc)
                t += 1

    nbh = _B * _H

    def step(i, s, extra=None, first=False):
        if first:
            issue_slices(len(stream))
        else:
            issue(u_kv(i + 1, (s + 1) % _NSLOT))
        wait_all(kv_buf.at[s], kv_sem.at[s])
        a_head(i, s)
        if extra is not None:
            extra()

    NPEEL = _NPEEL
    wait_all(bwuv_v, w_sem.at[S_BWUV])
    for i in range(NPEEL):
        step(i, i % _NSLOT, functools.partial(compute_ctx, i * 16 // NPEEL, (i + 1) * 16 // NPEEL), first=i == 0)

    def body(it, carry):
        for s in range(_NSLOT):
            step(it * _NSLOT + s, s)
        return carry

    NE = len(_END)
    ue = [u_end(e) for e in range(NE)]
    n_main = (nbh - 1) // _NSLOT
    jax.lax.fori_loop(NPEEL // _NSLOT, n_main, body, 0)
    for i in range(n_main * _NSLOT, nbh):
        s = i % _NSLOT
        if i + 1 < nbh:
            issue(u_kv(i + 1, (i + 1) % _NSLOT))
        else:
            issue(ue[0])
        wait_all(kv_buf.at[s], kv_sem.at[s])
        a_head(i, s)

    out_a = None
    out_b = None
    nxt = 1
    for e in range(NE):
        while nxt < min(e + 1 + _AHEAD[e], NE):
            issue(ue[nxt])
            nxt += 1
        h0, h1 = end_h[e], end_h[e + 1]
        wait_all(wob_v.at[:, pl.ds(h0 * _DH, (h1 - h0) * _DH)], w_sem.at[S_END + e])
        ta = out_proj(o_s, 0, h0, h1)
        tb = out_proj(ctx_s, 1, h0, h1)
        out_a = ta if out_a is None else out_a + ta
        out_b = tb if out_b is None else out_b + tb
    res = gate * out_a + (1.0 - gate) * out_b
    out_ref[...] = res[0:2, :].astype(_bf16)


@jax.jit
def pallas_gated_mix__mha_block_cached__compressed_kv_cla__decode_kernel(
    A_x: jax.Array,
    A_k_cache: jax.Array,
    A_v_cache: jax.Array,
    A_wq: jax.Array,
    A_wo: jax.Array,
    B_x: jax.Array,
    B_c_kv: jax.Array,
    B_w_q: jax.Array,
    B_w_uk: jax.Array,
    B_w_uv: jax.Array,
    B_w_o: jax.Array,
    gate_w: jax.Array,
):
    del B_x
    k3 = A_k_cache.reshape(_B * _H, _SK, _DH)
    v3 = A_v_cache.reshape(_B * _H, _SK, _DH)
    ckv = B_c_kv.reshape(_B * _SK, _DC)
    bwq = B_w_q.reshape(_D * _H, _DH)
    bwuk = B_w_uk.reshape(_DC * _H, _DH)
    bwuv = B_w_uv.reshape(_DC * _H, _DH)
    bwo = B_w_o.reshape(_H * _DH, _D)
    x2 = A_x.reshape(_B, _D)

    hbm = pl.BlockSpec(memory_space=pl.ANY)
    vmem = pl.BlockSpec(memory_space=pltpu.VMEM)
    V = pltpu.VMEM
    scratch = [
        V((_NSLOT, 2, _SK, _DH), _bf16),
        V((_D, _H * _DH), _bf16),
        V((2, _H * _DH, _D), _bf16),
        V((_NCK // _CPU, _B, _CPU, _SK // _NCK, _DC), _bf16),
        V((_D * _H, _DH), _bf16),
        V((_DC * _H, _DH), _bf16),
        V((_DC * _H, _DH), _bf16),
        V((_H, 8, _DH), _f32),
        V((_H, 8, _DH), _f32),
        V((_B, _H, _DC), _f32),
        V((_B, _H, _DC), _f32),
        V((_H, 8, _DH), _f32),
        V((_H, 8, _DH), _f32),
        V((_B, _H, 1), _f32),
        V((_B, _H, 1), _f32),
        V((_B, _H, _DC), _f32),
        V((_B, _D), _bf16),
        V((_D,), _bf16),
        pltpu.SemaphoreType.DMA((_NSLOT,)),
        pltpu.SemaphoreType.DMA((4 + _NCK // _CPU + len(_END),)),
        pltpu.SemaphoreType.DMA((2,)),
    ]
    out = pl.pallas_call(
        _kernel,
        out_shape=jax.ShapeDtypeStruct((_B, _D), _bf16),
        in_specs=[hbm] * 11,
        out_specs=vmem,
        scratch_shapes=scratch,
        compiler_params=pltpu.CompilerParams(vmem_limit_bytes=100 * 1024 * 1024),
    )(x2, gate_w, k3, v3, A_wq, A_wo, ckv, bwq, bwuk, bwuv, bwo)
    return out.reshape(_B, 1, _D)
```

```python
import functools

import jax
import jax.numpy as jnp
import jax.experimental.pallas as pl
import jax.experimental.pallas.tpu as pltpu

_B, _H, _SK, _DH, _D, _DC = 2, 32, 8192, 128, 512, 512

_PIECE_ROWS = 128
_VX_KV = 40
_NCK = 8
_CPU = 2
_LAG_C = 7
_END = (16, 8, 4, 2, 2)
_AHEAD = (1, 9, 9, 9, 9)
_PRE = (2, 4, 6)
_NPEEL = 6
_NSLOT = 2

_f32 = jnp.float32
_bf16 = jnp.bfloat16


def _dot(a, b):
    return jnp.dot(a, b, preferred_element_type=_f32)


def _dot_t(a, b):
    return jax.lax.dot_general(a, b, (((1,), (1,)), ((), ())), preferred_element_type=_f32)


def _unpack_pair(blk):
    lo = pltpu.bitcast(blk << 16, _f32).astype(_bf16)
    hi = pltpu.bitcast(blk & jnp.int32(-65536), _f32).astype(_bf16)
    return lo, hi


def _kernel(x_hbm, gw_hbm,
            k_hbm, v_hbm, wq_hbm, wo_hbm, ckv_hbm, bwq_hbm, bwuk_hbm, bwuv_hbm, bwo_hbm,
            out_ref,
            kv_buf, wq_v, wob_v, ckv_v, bwq_v, bwuk_v, bwuv_v,
            qa_s, qb_s, qlat_s, clat_s, o_s, ctx_s, m_s, l_s, acc_s,
            x_ref, gw_ref, w32, kv_sem, w_sem, x_sem):

    def rows(src, dst, nrow, n, sem, soff=0, doff=0):
        return [(src.at[pl.ds(soff + p * nrow, nrow)], dst.at[pl.ds(doff + p * nrow, nrow)], sem)
                for p in range(n)]

    def rot(u):
        n = len(u)
        if n % 64 == 0:
            return [u[(p // 64) * 64 + (p % 4) * 16 + (p % 64) // 4] for p in range(n)]
        if n % 32 == 0:
            return [u[(p // 32) * 32 + (p % 2) * 16 + (p % 32) // 2] for p in range(n)]
        return u

    def zip2(u, v, vx=0):
        v = [v[p ^ vx] for p in range(len(v))]
        out = []
        for a, b in zip(rot(u), rot(v)):
            out += [a + (0,), b + (1,)]
        return out

    def issue(unit, lo=0, hi=None):
        for p in range(lo, len(unit) if hi is None else hi):
            src, dst, sem, prio = unit[p]
            pltpu.make_async_copy(src, dst, sem).start(priority=prio)

    def wait_all(dst, sem):
        pltpu.make_async_copy(dst, dst, sem).wait()

    NCK, CPU = _NCK, _CPU
    CK = _SK // NCK
    NU = NCK // CPU
    S_WQ, S_BWQ, S_BWUK, S_BWUV = 0, 1, 2, 3
    S_CKV = 4
    S_END = S_CKV + NU

    u_wq = [(wq_hbm.at[pl.ds((p // 4) * 16, 16), pl.ds((p % 4) * 1024, 1024)],
             wq_v.at[pl.ds((p // 4) * 16, 16), pl.ds((p % 4) * 1024, 1024)], w_sem.at[S_WQ])
            for p in range(128)]
    u_w1 = zip2(u_wq, rows(bwq_hbm, bwq_v, 128, 128, w_sem.at[S_BWQ]))
    u_w2 = zip2(rows(bwuk_hbm, bwuk_v, 128, 128, w_sem.at[S_BWUK]),
                rows(bwuv_hbm, bwuv_v, 128, 128, w_sem.at[S_BWUV]))

    def u_ckv(u):
        streams = []
        for b in range(_B):
            st = []
            for c in range(u * CPU, (u + 1) * CPU):
                st += rows(ckv_hbm, ckv_v.at[u, b, c % CPU], 32, CK // 32, w_sem.at[S_CKV + u],
                           soff=b * _SK + c * CK)
            streams.append(st)
        return zip2(*streams)

    end_h = [0]
    for n in _END:
        end_h.append(end_h[-1] + n)

    def u_end(e):
        h0, n = end_h[e], _END[e]
        return zip2(*[rows(src, wob_v.at[j], 32, n * _DH // 32, w_sem.at[S_END + e], soff=h0 * _DH, doff=h0 * _DH)
                      for j, src in enumerate((wo_hbm, bwo_hbm))])

    def u_kv(i, slot):
        bh = (i % 2) * _H + i // 2
        n = _SK // _PIECE_ROWS
        return zip2(*[[(src.at[bh, pl.ds(p * _PIECE_ROWS, _PIECE_ROWS)],
                        kv_buf.at[slot, j, pl.ds(p * _PIECE_ROWS, _PIECE_ROWS)], kv_sem.at[slot])
                       for p in range(n)] for j, src in enumerate((k_hbm, v_hbm))], vx=_VX_KV)

    row8 = jax.lax.broadcasted_iota(jnp.int32, (8, _D), 0)
    scale_a = _DH ** -0.5
    scale_b = _DH ** -0.5

    def load_x8():
        xf = x_ref[...].astype(_f32)
        x0 = xf[0:1]
        x1 = xf[1:2]
        return jnp.where(row8 == 0, x0, jnp.where(row8 == 1, x1, 0.0))

    def compute_qa(x8):
        q = _dot(x8, wq_v[...]) * scale_a
        for h in range(_H):
            qa_s[h] = q[:, h * _DH:(h + 1) * _DH]

    def to_words(w_v, part=0, nparts=1):
        R = 256
        nblk = w32.shape[0] // R
        def cp(blk, c):
            w32[pl.ds(pl.multiple_of(blk * R, R), R), :] = pltpu.bitcast(
                w_v[pl.ds(pl.multiple_of(2 * blk * R, 2 * R), 2 * R), :], jnp.int32)
            return c
        jax.lax.fori_loop(part * nblk // nparts, (part + 1) * nblk // nparts, cp, 0)

    def compute_qb(x8, i0, i1):
        def pair_body(i, c):
            lo, hi = _unpack_pair(w32[pl.ds(i, _D, stride=_H // 2), :])
            qb_s[2 * i] = _dot(x8, lo)
            qb_s[2 * i + 1] = _dot(x8, hi)
            return c
        jax.lax.fori_loop(i0, i1, pair_body, 0)

    def compute_qlat(i0, i1):
        def pair_body(i, c):
            pair = _unpack_pair(w32[pl.ds(i, _DC, stride=_H // 2), :])
            for j in range(2):
                h = 2 * i + j
                ql = _dot_t(qb_s[h].astype(_bf16), pair[j]) * scale_b
                qlat_s[0, pl.ds(h, 1), :] = ql[0:1, :]
                qlat_s[1, pl.ds(h, 1), :] = ql[1:2, :]
            return c
        jax.lax.fori_loop(i0, i1, pair_body, 0)

    def b_chunk(b, c):
        first = c == 0
        last = c == NCK - 1
        ck = ckv_v[c // CPU, b, c % CPU]
        s = _dot_t(qlat_s[b].astype(_bf16), ck)
        m_cur = jnp.max(s, axis=-1, keepdims=True)
        if first:
            m_new = m_cur
        else:
            m_old = m_s[b]
            m_new = jnp.maximum(m_old, m_cur)
        p = jnp.exp(s - m_new)
        l_cur = jnp.sum(p, axis=-1, keepdims=True)
        pv = _dot(p.astype(_bf16), ck)
        if first:
            l_new, acc = l_cur, pv
        else:
            alpha = jnp.exp(m_old - m_new)
            l_new = alpha * l_s[b] + l_cur
            acc = alpha * acc_s[b] + pv
        if last:
            clat_s[b] = acc / l_new
        else:
            m_s[b] = m_new
            l_s[b] = l_new
            acc_s[b] = acc

    def compute_ctx(i0, i1):
        def pair_body(i, c):
            pair = _unpack_pair(w32[pl.ds(i, _DC, stride=_H // 2), :])
            for j in range(2):
                h = 2 * i + j
                r0 = clat_s[0, pl.ds(h, 1), :]
                r1 = clat_s[1, pl.ds(h, 1), :]
                lhs = jnp.where(row8 == 0, r0, jnp.where(row8 == 1, r1, 0.0))
                ctx_s[h] = _dot(lhs.astype(_bf16), pair[j])
            return c
        jax.lax.fori_loop(i0, i1, pair_body, 0)

    row8h = jax.lax.broadcasted_iota(jnp.int32, (8, _DH), 0)

    def a_head(i, slot):
        b = i % 2
        h = i // 2
        q8 = qa_s[h].astype(_bf16)
        s = _dot_t(q8, kv_buf[slot, 0])
        m = jnp.max(s, axis=-1, keepdims=True)
        p = jnp.exp(s - m)
        l = jnp.sum(p, axis=-1, keepdims=True)
        o = _dot(p.astype(_bf16), kv_buf[slot, 1]) / l
        o_s[h] = jnp.where(row8h == b, o, o_s[h])

    def out_proj(src_s, j, h0, h1):
        acc = None
        for h in range(h0, h1):
            t = _dot(src_s[h].astype(_bf16), wob_v[j, pl.ds(h * _DH, _DH), :])
            acc = t if acc is None else acc + t
        return acc

    cx = pltpu.make_async_copy(x_hbm, x_ref, x_sem.at[0])
    cg = pltpu.make_async_copy(gw_hbm, gw_ref, x_sem.at[1])
    cx.start()
    cg.start()
    issue(u_w1)
    o_s[...] = jnp.zeros_like(o_s)
    cx.wait()
    cg.wait()
    x8f = load_x8()
    x8 = x8f.astype(_bf16)
    gate = jax.nn.sigmoid(jnp.sum(x8f * gw_ref[...].astype(_f32).reshape(1, _D), axis=-1, keepdims=True))

    issue(u_w2, 0, 64)
    wait_all(wq_v, w_sem.at[S_WQ])
    compute_qa(x8)
    issue(u_w2, 64, 128)
    wait_all(bwq_v, w_sem.at[S_BWQ])
    to_words(bwq_v)
    issue(u_w2, 128, 192)
    compute_qb(x8, 0, 8)
    issue(u_w2, 192, 256)
    compute_qb(x8, 8, 16)

    stream = []
    for u in range(NU):
        stream += u_ckv(u)
    stream += u_kv(0, 0) + u_kv(1, 1)
    SL = CK // 32
    LAG = _LAG_C
    pos = 0

    def issue_slices(upto):
        nonlocal pos
        hi = min(upto * SL, len(stream))
        if hi > pos:
            issue(stream, pos, hi)
            pos = hi

    issue_slices(_PRE[0])
    wait_all(bwuk_v, w_sem.at[S_BWUK])
    to_words(bwuk_v)
    issue_slices(_PRE[1])
    compute_qlat(0, 8)
    issue_slices(_PRE[2])
    compute_qlat(8, 16)

    t = 0
    for u in range(NU):
        for cc in range(CPU):
            for b in range(_B):
                issue_slices(t + LAG)
                if cc == 0 and b == 0:
                    wait_all(ckv_v.at[u], w_sem.at[S_CKV + u])
                b_chunk(b, u * CPU + cc)
                t += 1

    nbh = _B * _H

    def step(i, s, extra=None, first=False):
        if first:
            issue_slices(len(stream))
        else:
            issue(u_kv(i + 1, (s + 1) % _NSLOT))
        wait_all(kv_buf.at[s], kv_sem.at[s])
        a_head(i, s)
        if extra is not None:
            extra()

    NPEEL = _NPEEL
    wait_all(bwuv_v, w_sem.at[S_BWUV])
    extras = [functools.partial(to_words, bwuv_v, 0, 2), functools.partial(to_words, bwuv_v, 1, 2)]
    extras += [functools.partial(compute_ctx, 4 * j, 4 * j + 4) for j in range(4)]
    assert len(extras) == NPEEL
    for i in range(NPEEL):
        step(i, i % _NSLOT, extras[i], first=i == 0)

    def body(it, carry):
        for s in range(_NSLOT):
            step(it * _NSLOT + s, s)
        return carry

    NE = len(_END)
    ue = [u_end(e) for e in range(NE)]
    n_main = (nbh - 1) // _NSLOT
    jax.lax.fori_loop(NPEEL // _NSLOT, n_main, body, 0)
    for i in range(n_main * _NSLOT, nbh):
        s = i % _NSLOT
        if i + 1 < nbh:
            issue(u_kv(i + 1, (i + 1) % _NSLOT))
        else:
            issue(ue[0])
        wait_all(kv_buf.at[s], kv_sem.at[s])
        a_head(i, s)

    out_a = None
    out_b = None
    nxt = 1
    for e in range(NE):
        while nxt < min(e + 1 + _AHEAD[e], NE):
            issue(ue[nxt])
            nxt += 1
        h0, h1 = end_h[e], end_h[e + 1]
        wait_all(wob_v.at[:, pl.ds(h0 * _DH, (h1 - h0) * _DH)], w_sem.at[S_END + e])
        ta = out_proj(o_s, 0, h0, h1)
        tb = out_proj(ctx_s, 1, h0, h1)
        out_a = ta if out_a is None else out_a + ta
        out_b = tb if out_b is None else out_b + tb
    res = gate * out_a + (1.0 - gate) * out_b
    out_ref[...] = res[0:2, :].astype(_bf16)


@jax.jit
def pallas_gated_mix__mha_block_cached__compressed_kv_cla__decode_kernel(
    A_x: jax.Array,
    A_k_cache: jax.Array,
    A_v_cache: jax.Array,
    A_wq: jax.Array,
    A_wo: jax.Array,
    B_x: jax.Array,
    B_c_kv: jax.Array,
    B_w_q: jax.Array,
    B_w_uk: jax.Array,
    B_w_uv: jax.Array,
    B_w_o: jax.Array,
    gate_w: jax.Array,
):
    del B_x
    k3 = A_k_cache.reshape(_B * _H, _SK, _DH)
    v3 = A_v_cache.reshape(_B * _H, _SK, _DH)
    ckv = B_c_kv.reshape(_B * _SK, _DC)
    bwq = B_w_q.reshape(_D * _H, _DH)
    bwuk = B_w_uk.reshape(_DC * _H, _DH)
    bwuv = B_w_uv.reshape(_DC * _H, _DH)
    bwo = B_w_o.reshape(_H * _DH, _D)
    x2 = A_x.reshape(_B, _D)

    hbm = pl.BlockSpec(memory_space=pl.ANY)
    vmem = pl.BlockSpec(memory_space=pltpu.VMEM)
    V = pltpu.VMEM
    scratch = [
        V((_NSLOT, 2, _SK, _DH), _bf16),
        V((_D, _H * _DH), _bf16),
        V((2, _H * _DH, _D), _bf16),
        V((_NCK // _CPU, _B, _CPU, _SK // _NCK, _DC), _bf16),
        V((_D * _H, _DH), _bf16),
        V((_DC * _H, _DH), _bf16),
        V((_DC * _H, _DH), _bf16),
        V((_H, 8, _DH), _f32),
        V((_H, 8, _DH), _f32),
        V((_B, _H, _DC), _f32),
        V((_B, _H, _DC), _f32),
        V((_H, 8, _DH), _f32),
        V((_H, 8, _DH), _f32),
        V((_B, _H, 1), _f32),
        V((_B, _H, 1), _f32),
        V((_B, _H, _DC), _f32),
        V((_B, _D), _bf16),
        V((_D,), _bf16),
        V((_D * _H // 2, _DH), jnp.int32),
        pltpu.SemaphoreType.DMA((_NSLOT,)),
        pltpu.SemaphoreType.DMA((4 + _NCK // _CPU + len(_END),)),
        pltpu.SemaphoreType.DMA((2,)),
    ]
    out = pl.pallas_call(
        _kernel,
        out_shape=jax.ShapeDtypeStruct((_B, _D), _bf16),
        in_specs=[hbm] * 11,
        out_specs=vmem,
        scratch_shapes=scratch,
        compiler_params=pltpu.CompilerParams(vmem_limit_bytes=100 * 1024 * 1024),
    )(x2, gate_w, k3, v3, A_wq, A_wo, ckv, bwq, bwuk, bwuv, bwo)
    return out.reshape(_B, 1, _D)
```
